```python
import os as _os
_os.environ.setdefault("JAX_PLATFORMS", "cpu")
import jax
import jax.numpy as jnp

def _softmax(x, axis=-1):
    return jax.nn.softmax(x, axis=axis)
def _gelu(x):
    return jax.nn.gelu(x, approximate=True)
def _silu(x):
    return jax.nn.silu(x)
def _sigmoid(x):
    return jax.nn.sigmoid(x)
def _layernorm(x, axis=-1, eps=1e-5):
    m = jnp.mean(x, axis=axis, keepdims=True)
    v = jnp.var(x, axis=axis, keepdims=True)
    return (x - m) / jnp.sqrt(v + eps)
def _scatter_add(tgt, idx, src, axis=0):
    return tgt.at[idx].add(src)
def _segment_sum(src, seg, n):
    return jax.ops.segment_sum(src, seg, n)
class _Rng:
    def __init__(self, key):
        self._k = key
    def _next(self):
        self._k, sub = jax.random.split(self._k)
        return sub
    def normal(self, shape):
        return jax.random.normal(self._next(), shape, dtype=jnp.bfloat16)
    def randint(self, lo, hi, shape):
        return jax.random.randint(self._next(), shape, lo, hi, dtype=jnp.int32)
    def uniform(self, shape, lo=0.0, hi=1.0):
        return jax.random.uniform(self._next(), shape, jnp.bfloat16, lo, hi)
    def permutation(self, n):
        return jax.random.permutation(self._next(), n)


kernel_name = 'gated_mix__ssm_conv_h3__linear_kernel_hedgehog__prompt'

def setup_inputs():
    _rng = _Rng(jax.random.key(int.from_bytes(__import__("os").urandom(4), "little")))
    _w = (lambda a: (lambda t: t.astype(jnp.bfloat16) if jnp.issubdtype(t.dtype, jnp.floating) else t)(jnp.asarray(a)))
    def _A_setup():
        B, S, D = 1, 2048, 576
        ks = 4
        return {
            "q": _w((lambda *s: _rng.normal(s) * 0.05)(B, S, D)),
            "k": _w((lambda *s: _rng.normal(s) * 0.4)(B, S, D)),
            "v": _w((lambda *s: _rng.normal(s) * 0.4)(B, S, D)),
            "shift_k": _w((lambda *s: _rng.normal(s) * 0.4)(D, ks) * 0.5),
            "ssm_k": _w((lambda *s: _rng.normal(s) * 0.4)(D, S) * (1.0 / S ** 0.5)),
            "ssm_D": _w((lambda *s: _rng.normal(s) * 0.4)(D)),
        }
    _A_in = _A_setup()

    def _B_setup():
        B, S, D, H = 1, 2048, 576, 32
        Dh = D // H
        return {
            "x": _w((lambda *s: _rng.normal(s) * 0.05)(B, S, D)),
            "wqkv": _w((lambda *s: _rng.normal(s) * 0.8)(D, 3 * D)),
            "w_phi": _w((lambda *s: _rng.normal(s) * 0.8)(H, Dh, Dh) * (Dh ** -0.5)),
            "wo": _w((lambda *s: _rng.normal(s) * 0.05)(D, D)),
        }
    _B_in = _B_setup()

    return {
        "A_q": _A_in["q"],
        "A_k": _A_in["k"],
        "A_v": _A_in["v"],
        "A_shift_k": _A_in["shift_k"],
        "A_ssm_k": _A_in["ssm_k"],
        "A_ssm_D": _A_in["ssm_D"],
        "B_x": _B_in["x"],
        "B_wqkv": _B_in["wqkv"],
        "B_w_phi": _B_in["w_phi"],
        "B_wo": _B_in["wo"],
        "gate_w": _w((lambda *s: _rng.normal(s) * 0.05)(576) * 16.0),
    }

def reference(A_q, A_k, A_v, A_shift_k, A_ssm_k, A_ssm_D, B_x, B_wqkv, B_w_phi, B_wo, gate_w):
    def _A_ref(q, k, v, shift_k, ssm_k, ssm_D):
        B, S, D = q.shape
        ks = shift_k.shape[-1]
        k_pad = jnp.pad(k, ((0, 0), (ks - 1, 0), (0, 0)))
        k_shift = jnp.zeros_like(k)
        for t in range(ks):
            k_shift = k_shift + k_pad[:, t:t + S, :] * shift_k[:, ks - 1 - t][None, None, :]
        kv = k_shift * v
        L = 2 * S
        kv_pad = jnp.pad(kv, ((0, 0), (0, S), (0, 0)))
        kf_pad = jnp.pad(ssm_k, ((0, 0), (0, S)))
        kv_f = (lambda x, axes=(-2,-1): jnp.fft.rfft2(x.astype(jnp.float32), axes=axes))(kv_pad[:, None, :, :], axes=(1, 2))
        kf_f = (lambda x, axes=(-2,-1): jnp.fft.rfft2(x.astype(jnp.float32), axes=axes))(kf_pad[:, None, :], axes=(1, 2))
        kf_f = (lambda x, *d: x.transpose(*d))(kf_f, 1, 2, 0)
        y_f = kv_f * kf_f[None, :, :, :]
        y = (lambda x, s, axes=(-2,-1): jnp.fft.irfft2(x, s=s, axes=axes).astype(jnp.bfloat16))(y_f, (1, L), axes=(1, 2))[:, 0, :S, :]
        y = y + kv * ssm_D[None, None, :]
        return q * y

    def _B_ref(x, wqkv, w_phi, wo):
        B, S, D = x.shape
        H = 32; Dh = D // H
        qkv = (lambda x, *d: x.transpose(*d))((x @ wqkv).reshape(B, S, 3, H, Dh), 2, 0, 3, 1, 4)
        q, k, v = qkv[0], qkv[1], qkv[2]
        pq = jnp.einsum("bhsd,hdf->bhsf", q, w_phi)
        pk = jnp.einsum("bhsd,hdf->bhsf", k, w_phi)
        phi_q = jnp.concatenate([_softmax(pq, axis=-1), _softmax(-pq, axis=-1)], axis=-1)
        phi_k = jnp.concatenate([_softmax(pk, axis=-1), _softmax(-pk, axis=-1)], axis=-1)
        kv = jnp.einsum("bhsf,bhsd->bhfd", phi_k, v)
        z  = jnp.einsum("bhsf->bhf", phi_k)
        num = jnp.einsum("bhqf,bhfd->bhqd", phi_q, kv)
        den = jnp.einsum("bhqf,bhf->bhq", phi_q, z)[..., None] + 1e-6
        o = num / den
        return (lambda x, *d: x.transpose(*d))(o, 0, 2, 1, 3).reshape(B, S, D) @ wo

    x = A_q
    g = _sigmoid((x * gate_w).sum(-1, keepdims=True))
    a = _A_ref(x, A_k, A_v, A_shift_k, A_ssm_k, A_ssm_D)
    b = _B_ref(x, B_wqkv, B_w_phi, B_wo)
    return g * a + (1 - g) * b
```

```python
import functools
import numpy as np
import jax
import jax.numpy as jnp
from jax import lax
import jax.experimental.pallas as pl
import jax.experimental.pallas.tpu as pltpu

S, D, H, DH = 2048, 576, 32, 18
C = 128
NCH = S // C
RB = 64
NA = D // RB
NSB = RB // 16
TS = 256
NT_ = TS // C
NB = S // TS
NG = 8
GR = 72
KT = 5
LOG2E = 1.4426950408889634
F32, BF16, U32 = jnp.float32, jnp.bfloat16, jnp.uint32

NN = (((1,), (0,)), ((), ()))
NT = (((1,), (1,)), ((), ()))


def _dot(a, b, dims=NN):
    return lax.dot_general(a, b, dims, preferred_element_type=F32)


def _pk(x):
    return pltpu.bitcast(x.astype(BF16), U32)


def _up(x):
    return pltpu.bitcast(x, BF16)


def _tree(op, xs):
    xs = list(xs)
    while len(xs) > 1:
        nxt = [op(xs[i], xs[i + 1]) for i in range(0, len(xs) - 1, 2)]
        if len(xs) % 2:
            nxt.append(xs[-1])
        xs = nxt
    return xs[0]


def _softmax_pair(p):
    ps = [p[8 * j:8 * j + 8] for j in range(9)]
    mx = _tree(jnp.maximum, ps)
    mn = _tree(jnp.minimum, ps)
    mx = jnp.maximum(mx, pltpu.roll(mx, 4, 0))
    mn = jnp.minimum(mn, pltpu.roll(mn, 4, 0))
    ep = [jnp.exp2(x - mx) for x in ps]
    en = [jnp.exp2(mn - x) for x in ps]
    sp = _tree(jnp.add, ep)
    sn = _tree(jnp.add, en)
    rp = pl.reciprocal(sp + pltpu.roll(sp, 4, 0), approx=True)
    rn = pl.reciprocal(sn + pltpu.roll(sn, 4, 0), approx=True)
    out = [pltpu.pack_elementwise([a * rp, b * rn], packed_dtype=BF16) for a, b in zip(ep, en)]
    return jnp.concatenate(out, axis=0).astype(U32)


def _load_wide(ref, r0, r1):
    rows = slice(r0 // 2, r1 // 2)
    return _up(jnp.concatenate([ref[t, rows, :] for t in range(KT - 1)] + [ref[KT - 1, rows, 0:64]], axis=1))


def _store_wide(ref, r0, r1, val):
    rows = slice(r0 // 2, r1 // 2)
    w = _pk(val)
    for t in range(KT - 1):
        ref[t, rows, :] = w[:, t * C:(t + 1) * C]
    ref[KT - 1, rows, 0:64] = w[:, (KT - 1) * C:D]


def _kernel(x_hbm, k_hbm, v_hbm, sh_hbm, h_hbm, d_hbm, wqkv_hbm, wphi_hbm, wo_hbm, gw_hbm,
            o_ref,
            x_v, k_v, v_v, h_v, sh_v, d_v, wqkv_v, wphi_v, wo_v, gw_v,
            f_v, col_v, wcat_v, wt_v, wot_v, uc_v, gc_v, y_v, phiq_v,
            g_v, kv_v, ot_v,
            sems):
    step = pl.program_id(0)
    never = lax.broadcasted_iota(jnp.int32, (8, C), 0) < -step

    def a_copies(i):
        rows = pl.ds(i * RB, RB)
        return [pltpu.make_async_copy(k_hbm.at[rows], k_v.at[rows], sems.at[16 + 3 * i]),
                pltpu.make_async_copy(v_hbm.at[rows], v_v.at[rows], sems.at[17 + 3 * i]),
                pltpu.make_async_copy(h_hbm.at[rows], h_v.at[rows], sems.at[18 + 3 * i])]

    def x_copy(i):
        return pltpu.make_async_copy(x_hbm.at[:, pl.ds(i * TS, TS)], x_v.at[i], sems.at[8 + i])

    small = [pltpu.make_async_copy(sh_hbm, sh_v, sems.at[0]),
             pltpu.make_async_copy(d_hbm, d_v, sems.at[1]),
             pltpu.make_async_copy(wphi_hbm, wphi_v, sems.at[2]),
             pltpu.make_async_copy(gw_hbm, gw_v, sems.at[3])]
    wqkv_cp = pltpu.make_async_copy(wqkv_hbm, wqkv_v, sems.at[4])
    wo_cp = pltpu.make_async_copy(wo_hbm, wo_v, sems.at[5])

    def fmat(e):
        return _up(jnp.concatenate([f_v[e, 0], f_v[e, 1]], axis=1))

    def a_fwd(i, rb):
        rows = pl.ds(pl.multiple_of(i * RB + 16 * rb, 16), 16)
        pr = slice(16 * rb, 16 * rb + 16)
        lane = lax.broadcasted_iota(jnp.int32, (16, C), 1)
        w = [col_v[j, rows, :] for j in range(4)]
        prev = [jnp.zeros((16, C), F32)] * 3
        us = []
        for c in range(NCH):
            kk = k_v[rows, c * C:(c + 1) * C].astype(F32)
            acc = kk * w[0]
            cur = []
            for j in range(1, 4):
                r = pltpu.roll(kk * w[j], j, 1)
                cur.append(r)
                acc = acc + jnp.where(lane < j, prev[j - 1], r)
            prev = cur
            us.append(acc * v_v[rows, c * C:(c + 1) * C].astype(F32))
        hts = []
        for e in range(2):
            cs = [e + 2 * t for t in range(8)]
            hts.append(_dot(jnp.concatenate([h_v[rows, c * C:(c + 1) * C] for c in cs], axis=0), fmat(e)))
        for c in range(NCH):
            t = c // 2
            hc = hts[c % 2][t * 16:(t + 1) * 16, 0:C]
            hd = hts[c % 2][t * 16:(t + 1) * 16, C:2 * C]
            if c == 0:
                gcr, gd = hc + col_v[4, rows, :], hd
            elif c % 2:
                gcr, gd = hc + pc, hd + pd
            else:
                gcr, gd = hc - pc, hd - pd
            gc_v[0, c, pr, :] = gcr
            gc_v[1, c, pr, :] = gd - gcr
            gc_v[2, c, pr, :] = gd + gcr
            pc, pd = hc, hd
        for e in range(2):
            cs = [e + 2 * t for t in range(8)]
            ft = _dot(jnp.concatenate([us[c] for c in cs], axis=0).astype(BF16), fmat(e))
            for t, c in enumerate(cs):
                a = ft[t * 16:(t + 1) * 16, 0:C]
                b = ft[t * 16:(t + 1) * 16, C:2 * C]
                uc_v[0, c, pr, :] = a
                uc_v[1, c, pr, :] = b
                uc_v[2, c, pr, :] = a + b

    def a_conv_inv(i, rb):
        res = {}
        link = None
        for hf in range(2):
            pr = slice(16 * rb + 8 * hf, 16 * rb + 8 * hf + 8)

            def chain(o, gq, uq, init, neg):
                acc = init
                for a in range(o + 1):
                    t = gc_v[gq, a, pr, :] * uc_v[uq, o - a, pr, :]
                    if acc is None:
                        acc = t if link is None else jnp.where(never, link[(o >> 1) & 1], t)
                    elif bool((a & 1) and ((o - a) & 1)) != neg:
                        acc = acc - t
                    else:
                        acc = acc + t
                return acc

            for o0 in (0, 1, 4, 5, 8, 9, 12, 13):
                nl = []
                for o in (o0, o0 + 2):
                    k1 = chain(o, 0, 2, None, False)
                    re = chain(o, 2, 1, k1, True)
                    im = chain(o, 1, 0, jnp.where(never, re, k1), False)
                    res[(o, hf)] = (re, im)
                    nl.append(im)
                link = nl
        for e in range(2):
            order = [(o0 + e + 2 * o2, hf) for hf in range(2) for o0 in (0, 4, 8, 12) for o2 in range(2)]
            lhs = jnp.concatenate(
                [jnp.concatenate([res[k][0] for k in order], axis=0),
                 jnp.concatenate([res[k][1] for k in order], axis=0)], axis=1).astype(BF16)
            yt = _dot(lhs, fmat(e), NT)
            for n_, (o, hf) in enumerate(order):
                rows = pl.ds(pl.multiple_of(i * RB + 16 * rb + 8 * hf, 8), 8)
                y_v[o, rows, :] = yt[8 * n_:8 * n_ + 8]

    @pl.when(step == 0)
    def _():
        for cp in small:
            cp.start()
        for cp in a_copies(0):
            cp.start()
        wqkv_cp.start()
        x_copy(0).start()
        for i in range(1, NA):
            for cp in a_copies(i):
                cp.start()
            if i < NB:
                x_copy(i).start()
        wo_cp.start()

        n = lax.broadcasted_iota(jnp.int32, (C, C), 0)
        f = lax.broadcasted_iota(jnp.int32, (C, C), 1)
        ang = (((2 * f + 1) * n) & 511).astype(F32) * (np.pi / 256)
        cs, sn = jnp.cos(ang), jnp.sin(ang)
        sg = (1 - 2 * (f & 1)).astype(F32)
        f_v[0, 0] = _pk(cs)
        f_v[0, 1] = _pk(-sn)
        f_v[1, 0] = _pk(-sg * sn)
        f_v[1, 1] = _pk(-sg * cs)
        er = lax.broadcasted_iota(jnp.int32, (D, D), 0)
        ec = lax.broadcasted_iota(jnp.int32, (D, D), 1)
        perm = (ec == 18 * (er & 31) + (er >> 5)).astype(BF16)
        kv_v[...] = jnp.zeros(kv_v.shape, F32)

        for cp in small:
            cp.wait()
        sh = sh_v[...].astype(F32)
        for j in range(4):
            col_v[j] = jnp.broadcast_to(sh[j:j + 1, :], (C, D)).T
        col_v[4] = jnp.broadcast_to(d_v[...].reshape(1, D).astype(F32), (C, D)).T

        for d in range(DH):
            wcat_v[:, 32 * d:32 * d + 32] = wphi_v[d].astype(F32)
        rr = lax.broadcasted_iota(jnp.int32, (GR, DH), 0)
        rc = lax.broadcasted_iota(jnp.int32, (GR, DH), 1)
        rep = (rr // 4 == rc).astype(BF16)
        wrep = _dot(rep, wcat_v[...].astype(BF16)).astype(BF16)
        t1 = _dot(wrep, perm)
        t1 = jnp.concatenate([t1, t1], axis=1)
        _store_wide(wt_v, 3 * D, 3 * D + 16,
                    jnp.broadcast_to(gw_v[...].reshape(1, D).astype(F32), (16, D)))

        for cp in a_copies(0):
            cp.wait()
        for rb in range(NSB):
            a_fwd(0, rb)

        wqkv_cp.wait()
        rowg = lax.broadcasted_iota(jnp.int32, (GR, C), 0) & 3
        colc = lax.broadcasted_iota(jnp.int32, (GR, C), 1)
        parts = {}
        for t in range(9):
            gs = [g for g in range(2 * NG) if GR * g < C * (t + 1) and GR * (g + 1) > C * t]
            tile = t1[:, t * C:(t + 1) * C]
            lhs = []
            for g in gs:
                lo = 18 * rowg + (GR * g - C * t)
                lhs.append(jnp.where((colc >= lo) & (colc < lo + 18), tile, 0.0))
            lhs = jnp.concatenate(lhs, axis=0).astype(BF16)
            res = _dot(lhs, wqkv_v[:, t * C:(t + 1) * C], NT)
            for n_, g in enumerate(gs):
                piece = res[n_ * GR:(n_ + 1) * GR]
                parts[g] = piece if g not in parts else parts[g] + piece
        for g in range(0, 2 * NG, 2):
            both = jnp.concatenate([parts[g], parts[g + 1]], axis=0) * LOG2E
            _store_wide(wt_v, GR * g, GR * (g + 2), both)
        _store_wide(wt_v, 2 * D, 3 * D, wqkv_v[:, 2 * D:3 * D].T)

    @pl.when((step >= 1) & (step <= NB))
    def _():
        i = step - 1
        x_copy(i).wait()
        for cp in a_copies(step):
            cp.wait()
        xs = [x_v[i, :, t * C:(t + 1) * C] for t in range(NT_)]
        ones = jnp.ones((8, TS), F32)

        def proj(r0, r1, t):
            return _dot(_load_wide(wt_v, r0, r1), xs[t])

        for r in range(4):
            pk = [proj(D + 2 * GR * r, D + 2 * GR * (r + 1), t) for t in range(NT_)]
            last = r == 3
            pv = [proj(2 * D + 2 * GR * r, 2 * D + 2 * GR * (r + 1) + (16 if last else 0), t) for t in range(NT_)]
            for t in range(NT_):
                p = proj(2 * GR * r, 2 * GR * (r + 1), t)
                for e in range(2):
                    phiq_v[i * NT_ + t, 2 * r + e] = _softmax_pair(p[GR * e:GR * (e + 1)])
                if last:
                    g_v[i * NT_ + t] = jax.nn.sigmoid(pv[t][2 * GR:2 * GR + 8])
            for e in range(2):
                phik = _up(jnp.concatenate(
                    [_softmax_pair(pk[t][GR * e:GR * (e + 1)]) for t in range(NT_)], axis=1))
                vext = jnp.concatenate(
                    [jnp.concatenate([pv[t][GR * e:GR * (e + 1)] for t in range(NT_)], axis=1), ones], axis=0)
                kv_v[2 * r + e] += _dot(vext.astype(BF16), phik, NT)
            a_conv_inv(i, r)
            a_fwd(step, r)

    @pl.when(step == NB + 1)
    def _():
        wo_cp.wait()
        r = lax.broadcasted_iota(jnp.int32, (80, 144), 0)
        c = (lax.broadcasted_iota(jnp.int32, (80, 144), 1) >> 1) & 3
        hr = jnp.where(r < GR, (r >= 18).astype(jnp.int32) + (r >= 36).astype(jnp.int32) + (r >= 54).astype(jnp.int32), r & 3)
        sub = lax.broadcasted_iota(jnp.int32, (8, C), 0)
        for gp in range(NG // 2):
            kvm = [jnp.where(hr == c, kv_v[2 * gp + e], 0.0).astype(BF16) for e in range(2)]
            for ct in range(NCH):
                os_ = []
                omg = 1.0 - g_v[ct]
                for e in range(2):
                    nd = _dot(kvm[e], _up(phiq_v[ct, 2 * gp + e]))
                    rd = omg * pl.reciprocal(nd[GR:GR + 8] + 1e-6, approx=True)
                    b = [jnp.broadcast_to(rd[j:j + 1], (8, C)) for j in range(4)]
                    pat = [b[0], b[0], jnp.where(sub < 2, b[0], b[1]), b[1], jnp.where(sub < 4, b[1], b[2]), b[2],
                           jnp.where(sub < 6, b[2], b[3]), b[3], b[3]]
                    os_ += [nd[8 * j:8 * j + 8] * pat[j] for j in range(9)]
                ot_v[ct, 2 * GR * gp:2 * GR * (gp + 1), :] = jnp.concatenate(os_, axis=0).astype(BF16)
            a_conv_inv(NA - 1, gp)
        _store_wide(wot_v, 0, D, wo_v[...].T)

    @pl.when(step > NB + 1)
    def _():
        i = step - (NB + 2)
        for t in range(NT_):
            ct = i * NT_ + t
            gs = jnp.concatenate([g_v[ct] * (1.0 / C)] * 2, axis=0)
            ot = ot_v[ct]
            for gp in range(4):
                bt = _dot(_load_wide(wot_v, 144 * gp, 144 * (gp + 1)), ot)
                for rb in range(9):
                    rows = slice(144 * gp + 16 * rb, 144 * gp + 16 * rb + 16)
                    o_ref[rows, t * C:(t + 1) * C] = (
                        bt[16 * rb:16 * rb + 16]
                        + (x_v[i, rows, t * C:(t + 1) * C].astype(F32) * gs) * y_v[ct, rows, :]).astype(BF16)


@jax.jit
def pallas_gated_mix__ssm_conv_h3__linear_kernel_hedgehog__prompt_kernel(A_q, A_k, A_v, A_shift_k, A_ssm_k, A_ssm_D, B_x, B_wqkv, B_w_phi, B_wo, gate_w):
    del B_x
    xt = jnp.transpose(A_q[0])
    kt = jnp.transpose(A_k[0])
    vt = jnp.transpose(A_v[0])
    sht = jnp.transpose(A_shift_k)
    wpt = jnp.transpose(B_w_phi, (1, 2, 0))
    out_t = pl.pallas_call(
        _kernel,
        grid=(2 + 2 * NB,),
        in_specs=[pl.BlockSpec(memory_space=pl.ANY)] * 10,
        out_specs=pl.BlockSpec((D, TS), lambda s: (0, jnp.maximum(s - (NB + 2), 0))),
        out_shape=jax.ShapeDtypeStruct((D, S), BF16),
        scratch_shapes=[
            pltpu.VMEM((NB, D, TS), BF16),
            pltpu.VMEM((D, S), BF16),
            pltpu.VMEM((D, S), BF16),
            pltpu.VMEM((D, S), BF16),
            pltpu.VMEM((4, D), BF16),
            pltpu.VMEM((D,), BF16),
            pltpu.VMEM((D, 3 * D), BF16),
            pltpu.VMEM((DH, DH, H), BF16),
            pltpu.VMEM((D, D), BF16),
            pltpu.VMEM((D,), BF16),
            pltpu.VMEM((2, 2, C // 2, C), U32),
            pltpu.VMEM((5, D, C), F32),
            pltpu.VMEM((DH, D), F32),
            pltpu.VMEM((KT, (3 * D + 16) // 2, C), U32),
            pltpu.VMEM((KT, D // 2, C), U32),
            pltpu.VMEM((3, NCH, RB, C), F32),
            pltpu.VMEM((3, NCH, RB, C), F32),
            pltpu.VMEM((NCH, D, C), F32),
            pltpu.VMEM((NCH, NG, GR, C), U32),
            pltpu.VMEM((NCH, 8, C), F32),
            pltpu.VMEM((NG, 80, 2 * GR), F32),
            pltpu.VMEM((NCH, D, C), BF16),
            pltpu.SemaphoreType.DMA((16 + 3 * NA,)),
        ],
        compiler_params=pltpu.CompilerParams(
            dimension_semantics=("arbitrary",), vmem_limit_bytes=100 * 1024 * 1024),
    )(xt, kt, vt, sht, A_ssm_k, A_ssm_D, B_wqkv, wpt, B_wo, gate_w)
    return jnp.transpose(out_t)[None]
```

```python
import os
import numpy as np
import jax
import jax.numpy as jnp
from jax import lax
import jax.experimental.pallas as pl
import jax.experimental.pallas.tpu as pltpu

S, D, H, DH = 2048, 576, 32, 18
C = 128
NCH = S // C
SKEW = 3
TS = 256
NT_ = TS // C
NB = S // TS
NG = 8
GR = 72
KT = 5
OB = 144
LOG2E = 1.4426950408889634
F32, BF16, U32 = jnp.float32, jnp.bfloat16, jnp.uint32
ENV = os.environ.get
ORDER = ENV("ORDER", "K0 K1 V0 V1 Q0 Q1 IN KB FH KA FU").split()
GATE = ENV("GATE", "FH")
ONLY = ENV("ONLY", "012345")
OLAG = int(ENV("OLAG", "3"))
INPOS = [int(v) for v in ENV('INPOS', '6 10 14 18').split()]
FOFF = int(ENV('FOFF', '0'))
GATE2 = int(ENV('GATE2', '0'))
PG = dict(kv.split(':') for kv in ENV('PG', '8:K1').split())
ORDER0 = ENV('ORDER0', 'K0 K1 Q0 K2 Q1 K3 Q2 W Q3 FH0 FH1 V0 FU0 V1 KV0 FU1 V2 KV1 V3 KV2 FU2 KV3 FH2').split()
MERGE = int(ENV('MERGE', '3'))
OBS = [int(v) for v in ENV('OBS', '0 144 384 512 576').split()]
UG = ENV('UG', '')
PORDER = (0, 1, 4, 5, 8, 9, 12, 13)
WK0, WQ0, WV0, WROWS = 0, 576, 1088, 1680

NN = (((1,), (0,)), ((), ()))
NT = (((1,), (1,)), ((), ()))
TN = (((0,), (0,)), ((), ()))


def _dot(a, b, dims=NN):
    return lax.dot_general(a, b, dims, preferred_element_type=F32)


def _pk(x):
    return pltpu.bitcast(x.astype(BF16), U32)


def _up(x):
    return pltpu.bitcast(x, BF16)


def _iota(shape, dim):
    return lax.broadcasted_iota(jnp.int32, shape, dim)


def _tree(op, xs):
    xs = list(xs)
    while len(xs) > 1:
        nxt = [op(xs[i], xs[i + 1]) for i in range(0, len(xs) - 1, 2)]
        if len(xs) % 2:
            nxt.append(xs[-1])
        xs = nxt
    return xs[0]


def _softmax_pair(p, last):
    ps = [p[8 * j:8 * j + 8] for j in range(8)] + [last]
    mx = _tree(jnp.maximum, ps)
    mn = _tree(jnp.minimum, ps)
    mx = jnp.maximum(mx, pltpu.roll(mx, 4, 0))
    mn = jnp.minimum(mn, pltpu.roll(mn, 4, 0))
    ep = [jnp.exp2(x - mx) for x in ps]
    en = [jnp.exp2(mn - x) for x in ps]
    sp = _tree(jnp.add, ep)
    sn = _tree(jnp.add, en)
    rp = pl.reciprocal(sp + pltpu.roll(sp, 4, 0), approx=True)
    rn = pl.reciprocal(sn + pltpu.roll(sn, 4, 0), approx=True)
    out = [pltpu.pack_elementwise([a * rp, b * rn], packed_dtype=BF16) for a, b in zip(ep, en)]
    return jnp.concatenate(out, axis=0).astype(U32)


def _load_wide(ref, r0, r1, full=False):
    rows = slice(r0 // 2, r1 // 2)
    last = ref[KT - 1, rows, :] if full else ref[KT - 1, rows, 0:64]
    return _up(jnp.concatenate([ref[t, rows, :] for t in range(KT - 1)] + [last], axis=1))


def _store_wide(ref, r0, r1, val):
    rows = slice(r0 // 2, r1 // 2)
    w = _pk(val)
    for t in range(KT - 1):
        ref[t, rows, :] = w[:, t * C:(t + 1) * C]
    ref[KT - 1, rows, 0:64] = w[:, (KT - 1) * C:D]


def _kernel(x_hbm, k_hbm, v_hbm, sh_hbm, h_hbm, d_hbm, wqkv_hbm, wphi_hbm, wo_hbm, gw_hbm,
            o_hbm,
            x_v, k_v, v_v, h_v, sh_v, d_v, wqk_v, wv_v, wphi_v, wo_v, gw_v,
            f_v, col_v, wcat_v, wt_v, wot_v, ab0, ab1, ab2, ab3, y_v, phiq_v, phik_v,
            g_v, kv_v, kvl_v, ot_v, dp_v, zl_v, cb_v, o_v,
            sems):
    step = pl.program_id(0)
    ab_l = [ab0, ab1, ab2, ab3]
    never = _iota((8, C), 0) < -step
    glink = [None]
    sub = _iota((8, C), 0)

    def gate(tok):
        if glink[0] is not None:
            glink[0] = jnp.where(never, tok, glink[0])

    def a_copies(sem, start, size):
        rows = pl.ds(start, size)
        return [pltpu.make_async_copy(src.at[rows], dst.at[rows], sems.at[sem])
                for src, dst in ((k_hbm, k_v), (v_hbm, v_v), (h_hbm, h_v))]

    def x_copy(sem, i):
        return pltpu.make_async_copy(x_hbm.at[:, pl.ds(i * TS, TS)], x_v.at[i], sems.at[sem])

    def wqk_copy(sem, c):
        return pltpu.make_async_copy(wqkv_hbm.at[:, pl.ds(3 * C * c, 3 * C)], wqk_v.at[c], sems.at[sem])

    cp_small = [pltpu.make_async_copy(src, dst, sems.at[0])
                for src, dst in ((wphi_hbm, wphi_v), (sh_hbm, sh_v), (d_hbm, d_v), (gw_hbm, gw_v))]
    cp_w0 = [wqk_copy(1, 0)]
    cp_w1 = [wqk_copy(2, 1)]
    cp_w2 = [wqk_copy(3, 2), x_copy(3, 0)]
    cp_w3 = [pltpu.make_async_copy(wqkv_hbm.at[:, pl.ds(2 * D, D)], wv_v, sems.at[4])] + a_copies(4, 0, 16 * SKEW)

    def cp_step(s):
        return [x_copy(4 + s, s)] + a_copies(4 + s, pl.multiple_of(16 * SKEW + (s - 1) * 64, 16), 64)

    a_done = 16 * SKEW + (NB - 1) * 64
    cp_last = a_copies(4 + NB, a_done, D - a_done) + [pltpu.make_async_copy(wo_hbm, wo_v, sems.at[4 + NB])]

    def wait(cps):
        for cp in cps:
            cp.wait()

    def fmat(e):
        return _up(jnp.concatenate([f_v[e, 0], f_v[e, 1]], axis=1))

    def a_fwd_h(n, ab):
        rows = pl.ds(pl.multiple_of(n * 16, 16), 16)
        hts = []
        for e in range(2):
            cs = [e + 2 * t for t in range(8)]
            hts.append(_dot(jnp.concatenate([h_v[rows, c * C:(c + 1) * C] for c in cs], axis=0), fmat(e)))
        for c in range(NCH):
            t = c // 2
            hc = hts[c % 2][t * 16:(t + 1) * 16, 0:C]
            hd = hts[c % 2][t * 16:(t + 1) * 16, C:2 * C]
            if c == 0:
                gcr, gd = hc + col_v[4, rows, :], hd
            elif c % 2:
                gcr, gd = hc + pc, hd + pd
            else:
                gcr, gd = hc - pc, hd - pd
            ab[3, c] = gcr
            ab[4, c] = gd - gcr
            ab[5, c] = gd + gcr
            pc, pd = hc, hd
        return hts[0][0:8, 0:C]

    def a_fwd_u(n, ab, tok=None):
        rows = pl.ds(pl.multiple_of(n * 16, 16), 16)
        lane = _iota((16, C), 1)
        w = [col_v[j, rows, :] for j in range(4)]
        if tok is not None:
            w = [jnp.concatenate([jnp.where(never, tok, x[0:8]), jnp.where(never, tok, x[8:16])], axis=0) for x in w]
        prev = [jnp.zeros((16, C), F32)] * 3
        us = []
        for c in range(NCH):
            kk = k_v[rows, c * C:(c + 1) * C].astype(F32)
            acc = kk * w[0]
            cur = []
            for j in range(1, 4):
                r = pltpu.roll(kk * w[j], j, 1)
                cur.append(r)
                acc = acc + jnp.where(lane < j, prev[j - 1], r)
            prev = cur
            us.append(acc * v_v[rows, c * C:(c + 1) * C].astype(F32))
        for e in range(2):
            cs = [e + 2 * t for t in range(8)]
            ft = _dot(jnp.concatenate([us[c] for c in cs], axis=0).astype(BF16), fmat(e))
            for t, c in enumerate(cs):
                a = ft[t * 16:(t + 1) * 16, 0:C]
                b = ft[t * 16:(t + 1) * 16, C:2 * C]
                ab[0, c] = a
                ab[1, c] = b
                ab[2, c] = a + b
        return ft[0:8, 0:C]

    def a_conv_inv(n, ab, gates=None):
        res = {}
        link = glink[0]
        for hf in range(2):
            pr = slice(8 * hf, 8 * hf + 8)

            def chain(o, gq, uq, acc, neg):
                for a in range(o + 1):
                    t = ab[gq, a, pr, :] * ab[uq, o - a, pr, :]
                    if acc is None:
                        acc = t if link is None else jnp.where(never, link, t)
                    elif bool((a & 1) and ((o - a) & 1)) != neg:
                        acc = acc - t
                    else:
                        acc = acc + t
                return acc

            for pi, o0 in enumerate(PORDER):
                os_ = (o0, o0 + 2)
                if gates and (8 * hf + pi) in gates:
                    tk = gates[8 * hf + pi]
                    link = tk if link is None else jnp.where(never, tk, link)
                k1 = [chain(o, 3, 2, None, False) for o in os_]
                re = [chain(o, 5, 1, k, True) for o, k in zip(os_, k1)]
                rep = pltpu.pack_elementwise(re, packed_dtype=BF16)
                link = pltpu.bitcast(rep, F32)
                k1 = [jnp.where(never, link, k) for k in k1]
                im = [chain(o, 4, 0, k, False) for o, k in zip(os_, k1)]
                imp = pltpu.pack_elementwise(im, packed_dtype=BF16)
                link = pltpu.bitcast(imp, F32)
                res[(o0, hf)] = (rep, imp)
        glink[0] = link
        for e in range(2):
            order = [(o0, hf) for hf in range(2) for o0 in PORDER if (o0 & 1) == e]
            lhs = _up(jnp.concatenate(
                [jnp.concatenate([res[k][0] for k in order], axis=0),
                 jnp.concatenate([res[k][1] for k in order], axis=0)], axis=1))
            yt = _dot(lhs, fmat(e), NT)
            for n_, (o0, hf) in enumerate(order):
                rows = pl.ds(pl.multiple_of(n * 32 + 16 * hf, 16), 16)
                y_v[(o0 >> 2) * 2 + (o0 & 1), rows, :] = yt[16 * n_:16 * n_ + 16]
        return yt[0:8]

    def feat(p, shared):
        return [_softmax_pair(p[0:64], jnp.where(sub < 4, shared, 0.0)),
                _softmax_pair(p[64:128], jnp.where(sub < 4, 0.0, shared))]

    def proj(xs, r0, r1, t):
        return _dot(_load_wide(wt_v, r0, r1), xs[t])

    def k_unit(xs, r, t):
        p = proj(xs, WK0 + 144 * r, WK0 + 144 * (r + 1), t)
        return feat(p[16:144], p[0:8]), p[8:16]

    def q_unit(xs, i, r, t, sq):
        p = proj(xs, WQ0 + 128 * r, WQ0 + 128 * (r + 1), t)
        for e, ph in enumerate(feat(p, sq)):
            phiq_v[i * NT_ + t, 2 * r + e] = ph
        return p[0:8], pltpu.bitcast(ph[64:72], F32)

    def v_unit(xs, i, r, t):
        p = proj(xs, WV0 + 144 * r, WV0 + 144 * (r + 1) + (16 if r == 3 else 0), t)
        if r == 3:
            g_v[i * NT_ + t] = jax.nn.sigmoid(p[2 * GR:2 * GR + 8])
        return p

    def kv_unit(g, pks, pvs, first=False):
        e = g % 2
        phik = _up(jnp.concatenate(pks, axis=1))
        vb = jnp.concatenate(
            [jnp.concatenate([p[GR * e:GR * (e + 1)] for p in pvs], axis=1), jnp.ones((8, TS), F32)],
            axis=0).astype(BF16)
        a = _dot(vb, phik[0:C], NT)
        b = _dot(phik[C:2 * GR], vb, NT)
        if first:
            kv_v[g] = a
            kvl_v[g] = b
        else:
            kv_v[g] += a
            kvl_v[g] += b

    def out_unit(j, ct):
        ra, rb_ = OBS[j], OBS[j + 1]
        gs = jnp.concatenate([g_v[ct] * (1.0 / C)] * 2, axis=0)
        bt = _dot(_load_wide(wot_v, ra, rb_, full=True), ot_v[ct])
        for r0 in range(ra, rb_, 16):
            y = y_v[(ct >> 2) * 2 + (ct & 1), pl.ds(2 * r0 + ((ct >> 1) & 1), 16, stride=2), :]
            xq = x_v[ct // NT_, r0:r0 + 16, (ct % NT_) * C:(ct % NT_ + 1) * C].astype(F32)
            o_v[r0:r0 + 16, ct * C:(ct + 1) * C] = (bt[r0 - ra:r0 - ra + 16] + (xq * gs) * y).astype(BF16)
        return bt[0:8]

    def out_copy(j):
        rows = pl.ds(OBS[j], OBS[j + 1] - OBS[j])
        return pltpu.make_async_copy(o_v.at[rows], o_hbm.at[rows], sems.at[5 + NB + j])

    @pl.when(step == 0)
    def _():
        for cp in cp_small + cp_w0 + cp_w1 + cp_w2 + cp_w3:
            cp.start()
        for s in range(1, NB):
            for cp in cp_step(s):
                cp.start()
        for cp in cp_last:
            cp.start()
        if "0" not in ONLY:
            wait(cp_small + cp_w0 + cp_w1 + cp_w2 + cp_w3)
            return

        n = _iota((C, C), 0)
        f = _iota((C, C), 1)
        ang = (((2 * f + 1) * n) & 511).astype(F32) * (np.pi / 256)
        cs, sn = jnp.cos(ang), jnp.sin(ang)
        sg = (1 - 2 * (f & 1)).astype(F32)
        f_v[0, 0] = _pk(cs)
        f_v[0, 1] = _pk(-sn)
        f_v[1, 0] = _pk(-sg * sn)
        f_v[1, 1] = _pk(-sg * cs)
        er = _iota((D, D), 0)
        ec = _iota((D, D), 1)
        perm = (ec == 18 * (er & 31) + (er >> 5)).astype(BF16)
        dp_v[...] = jnp.zeros(dp_v.shape, F32)

        wait(cp_small)
        for d in range(DH):
            wcat_v[:, 32 * d:32 * d + 32] = wphi_v[d].astype(F32)
        rep = (_iota((GR, DH), 0) // 4 == _iota((GR, DH), 1)).astype(BF16)
        wrep = _dot(rep, wcat_v[...].astype(BF16)).astype(BF16)
        t1 = _dot(wrep, perm)
        t1 = jnp.concatenate([t1, t1], axis=1)
        _store_wide(wt_v, WV0 + D, WROWS, jnp.broadcast_to(gw_v[...].reshape(1, D).astype(F32), (16, D)))

        rowg = _iota((GR, C), 0) & 3
        colc = _iota((GR, C), 1)
        lo4 = _iota((8, D), 0) < 4
        parts, d16 = {}, {}

        def fold(t):
            gs = [g for g in range(2 * NG) if GR * g < C * (t + 1) and GR * (g + 1) > C * t]
            tile = t1[:, t * C:(t + 1) * C]
            lhs = []
            for g in gs:
                lo = 18 * rowg + (GR * g - C * t)
                lhs.append(jnp.where((colc >= lo) & (colc < lo + 18), tile, 0.0))
            lhs = jnp.concatenate(lhs, axis=0).astype(BF16)
            res = _dot(lhs, wqk_v[t // 3, :, (t % 3) * C:(t % 3 + 1) * C], NT)
            for n_, g in enumerate(gs):
                piece = res[n_ * GR:(n_ + 1) * GR]
                parts[g] = piece if g not in parts else parts[g] + piece
                if GR * (g + 1) <= C * (t + 1):
                    w = parts[g] * LOG2E
                    tail = w[64:72]
                    swap = pltpu.roll(tail, 4, 0)
                    w17 = jnp.where(lo4, swap, tail)
                    main = jnp.concatenate([w[8 * j:8 * j + 8] - w17 for j in range(8)], axis=0)
                    d16[g] = (tail - swap) if g % 2 == 0 else (swap - tail)
                    if g < NG:
                        r0 = WQ0 + 64 * g
                    else:
                        r0 = WK0 + 144 * ((g - NG) // 2) + 16 + 64 * (g % 2)
                    _store_wide(wt_v, r0, r0 + 64, main)
                    if g >= NG and g % 2 == 1:
                        r0 = WK0 + 144 * ((g - NG) // 2)
                        _store_wide(wt_v, r0, r0 + 16, jnp.concatenate(
                            [jnp.where(lo4, d16[g - 1], d16[g]), jnp.where(lo4, d16[g - 1 - NG], d16[g - NG])], axis=0))

        wait(cp_w0)
        for t in range(0, 3):
            fold(t)
        wait(cp_w1)
        for t in range(3, 6):
            fold(t)
        wait(cp_w2)
        for t in range(6, 9):
            fold(t)
        sh = sh_v[...].astype(F32)
        for j in range(4):
            col_v[j] = jnp.broadcast_to(sh[j:j + 1, :], (C, D)).T
        col_v[4] = jnp.broadcast_to(d_v[...].reshape(1, D).astype(F32), (C, D)).T
        xs = [x_v[0, :, t * C:(t + 1) * C] for t in range(NT_)]
        sq, pv = {}, {}
        for u in ORDER0:
            if u == "W":
                wait(cp_w3)
                _store_wide(wt_v, WV0, WV0 + D, wv_v[...].T)
                xs = [x_v[0, :, t * C:(t + 1) * C] for t in range(NT_)]
                continue
            r = int(u[-1])
            if u[:-1] == "K":
                for t in range(NT_):
                    pk, sq[r, t] = k_unit(xs, r, t)
                    for e in range(2):
                        phik_v[2 * r + e, t] = pk[e]
            elif u[:-1] == "Q":
                for t in range(NT_):
                    q_unit(xs, 0, r, t, sq[r, t])
            elif u[:-1] == "V":
                pv[r] = [v_unit(xs, 0, r, t) for t in range(NT_)]
            elif u[:-1] == "KV":
                for g in (2 * r, 2 * r + 1):
                    kv_unit(g, [phik_v[g, t] for t in range(NT_)], pv[r], first=True)
            elif u[:-1] == "FH":
                a_fwd_h(r, ab_l[r])
            elif u[:-1] == "FU":
                a_fwd_u(r, ab_l[r])

    @pl.when((step >= 1) & (step < NB))
    def _():
        i = step
        wait(cp_step(step))
        if "1" not in ONLY:
            return
        glink[0] = None
        xs = [x_v[i, :, t * C:(t + 1) * C] for t in range(NT_)]
        n0 = 4 * (step - 1)
        for r in range(4):
            pk, pv, sq, toks = {}, {}, {}, {}
            for u in ORDER:
                tok = None
                if u[0] == "K" and u[1] in "01":
                    pk[int(u[1])], sq[int(u[1])] = k_unit(xs, r, int(u[1]))
                    toks[u] = sq[int(u[1])]
                    toks["s" + u] = pltpu.bitcast(pk[int(u[1])][1][64:72], F32)
                elif u[0] == "V":
                    pv[int(u[1])] = v_unit(xs, i, r, int(u[1]))
                    toks[u] = pv[int(u[1])][0:8]
                    toks["e" + u] = pv[int(u[1])][136:144]
                elif u[0] == "Q":
                    toks[u], toks["s" + u] = q_unit(xs, i, r, int(u[1]), sq[int(u[1])])
                elif u in ("KA", "KB"):
                    e = 0 if u == "KA" else 1
                    kv_unit(2 * r + e, [pk[t][e] for t in range(NT_)], [pv[t] for t in range(NT_)])
                elif u == "FH":
                    tok = toks[u] = a_fwd_h(n0 + r + SKEW, ab_l[(r + SKEW) % 4])
                elif u == "FU":
                    tok = toks[u] = a_fwd_u(n0 + r + SKEW, ab_l[(r + SKEW) % 4], toks.get(UG))
                elif u == "IN":
                    tok = toks[u] = a_conv_inv(n0 + r, ab_l[r], {int(k): toks[v] for k, v in PG.items()})
                    toks['CV'] = glink[0]
                if u == GATE:
                    gate(tok)

    N2 = 4 * (NB - 1)

    def blk1():
        if MERGE < 3:
            glink[0] = None
        for ct in range(NCH):
            out_unit(1, ct)
            if ct == 3:
                a_fwd_h(N2 + 4 + SKEW, ab_l[SKEW % 4])
                a_fwd_u(N2 + 4 + SKEW, ab_l[SKEW % 4])
            if ct in (7, 14):
                a_conv_inv(N2 + 4 + ct // 8, ab_l[ct // 8])
        out_copy(1).start()

    def blk2():
        if MERGE == 0:
            glink[0] = None
        for ct in range(NCH):
            out_unit(2, ct)
            if ct in (7, 14):
                a_conv_inv(N2 + 6 + ct // 8, ab_l[2 + ct // 8])
        out_copy(2).start()

    def blk3():
        for ct in range(NCH):
            out_unit(3, ct)
        out_copy(3).start()
        for j in range(4):
            out_copy(j).wait()

    @pl.when(step == NB)
    def _():
        wait(cp_last)
        if "2" not in ONLY:
            return
        glink[0] = None

        def head_of(v):
            return (v >= 18).astype(jnp.int32) + (v >= 36).astype(jnp.int32) + (v >= 54).astype(jnp.int32)

        r = _iota((80, C), 0)
        hr = jnp.where(r < GR, head_of(r), r & 3)
        mmask = hr == ((_iota((80, C), 1) >> 1) & 3)
        ll = _iota((8, 80), 1)
        lmask = (head_of(ll) == (_iota((8, 80), 0) >> 1)) & (ll < GR)
        sc = _iota((8, 2 * C), 1)
        sel = ((sc >= C) | ((sc & 1) == (_iota((8, 2 * C), 0) & 1))).astype(BF16)
        a_fwd_h(N2 + SKEW, ab_l[SKEW % 4])
        kvm = []
        for g in range(NG):
            kvl = kvl_v[g]
            h16, h17 = (kvl[0:8], kvl[8:16]) if g % 2 == 0 else (kvl[8:16], kvl[0:8])
            k17 = jnp.where(lmask, h17, 0.0).astype(BF16)
            tt = _dot(k17, sel, TN)
            kvm.append(jnp.where(mmask, kv_v[g] - tt[:, 0:C], 0.0).astype(BF16))
            cb_v[g] = tt[0:GR, C:2 * C]
            dd = jnp.where(lmask, h16 - k17.astype(F32), 0.0)
            dp_v[g // 2, 8 * (g % 2):8 * (g % 2) + 8, GR * (g % 2):GR * (g % 2) + GR] = dd[:, 0:GR]
            zl_v[g] = jnp.broadcast_to(kvl[:, GR:GR + 1], (16, C))
        m16 = [_dot(dp_v[r_].astype(BF16), wo_v[144 * r_:144 * (r_ + 1), :]) for r_ in range(4)]
        a_fwd_u(N2 + SKEW, ab_l[SKEW % 4])
        wlast = jnp.concatenate([wo_v[4 * C:D, :].astype(F32)] + m16, axis=0)
        wot_v[KT - 1] = _pk(wlast.T)
        w4 = pltpu.bitcast(wo_v[0:4 * C, :].T, U32)
        for t in range(KT - 1):
            wot_v[t] = w4[:, t * C:(t + 1) * C]

        def num_unit(ct):
            omg = 1.0 - g_v[ct]
            for gp in range(NG // 2):
                os_, xs_ = [], []
                for e in range(2):
                    g = 2 * gp + e
                    nd = _dot(kvm[g], _up(phiq_v[ct, g, 0:64, :]))
                    pl_ = phiq_v[ct, g, 64:72, :]
                    ph = [pltpu.unpack_elementwise(pl_, index=sg_, packed_dtype=BF16, unpacked_dtype=F32)
                          for sg_ in range(2)]
                    dl = (ph[0] * zl_v[g, pl.ds(0, 8, stride=2), :] + ph[1] * zl_v[g, pl.ds(1, 8, stride=2), :])
                    den = nd[GR:GR + 8] + (dl + pltpu.roll(dl, 4, 0)) + 1e-6
                    rd = omg * pl.reciprocal(den, approx=True)
                    b = [jnp.broadcast_to(rd[j:j + 1], (8, C)) for j in range(4)]
                    pat = [b[0], b[0], jnp.where(sub < 2, b[0], b[1]), b[1], jnp.where(sub < 4, b[1], b[2]), b[2],
                           jnp.where(sub < 6, b[2], b[3]), b[3], b[3]]
                    os_ += [(nd[8 * j:8 * j + 8] + cb_v[g, 8 * j:8 * j + 8, :]) * pat[j] for j in range(9)]
                    xs_.append((ph, rd))
                ot_v[ct, 2 * GR * gp:2 * GR * (gp + 1), :] = jnp.concatenate(os_, axis=0).astype(BF16)
                rd = jnp.where(sub < 4, xs_[0][1], xs_[1][1])
                xx = [jnp.where(sub < 4, xs_[0][0][sg_], xs_[1][0][sg_]) * rd for sg_ in range(2)]
                ot_v[ct, D + 16 * gp:D + 16 * (gp + 1), :] = _up(pltpu.pack_elementwise(xx, packed_dtype=BF16))

        nstep = NCH + OLAG
        for it in range(nstep):
            if it < NCH:
                num_unit(it)
            if it >= OLAG:
                out_unit(0, it - OLAG)
            for r_ in range(4):
                if it == INPOS[r_]:
                    a_conv_inv(N2 + r_, ab_l[r_])
                if r_ < 3 and it == INPOS[r_] + FOFF:
                    tok = a_fwd_h(N2 + r_ + 1 + SKEW, ab_l[(r_ + 1 + SKEW) % 4])
                    if GATE2:
                        gate(tok)
                    a_fwd_u(N2 + r_ + 1 + SKEW, ab_l[(r_ + 1 + SKEW) % 4])
        out_copy(0).start()
        if MERGE >= 3:
            blk1()
            blk2()
            blk3()

    if MERGE == 0:
        pl.when(step == NB + 1)(blk1)
        pl.when(step == NB + 2)(blk2)
        pl.when(step == NB + 3)(blk3)
    elif MERGE == 1:
        @pl.when(step == NB + 1)
        def _():
            blk1()
            blk2()
        pl.when(step == NB + 2)(blk3)
    elif MERGE == 2:
        @pl.when(step == NB + 1)
        def _():
            blk1()
            blk2()
            blk3()


@jax.jit
def pallas_gated_mix__ssm_conv_h3__linear_kernel_hedgehog__prompt_kernel(A_q, A_k, A_v, A_shift_k, A_ssm_k, A_ssm_D, B_x, B_wqkv, B_w_phi, B_wo, gate_w):
    del B_x
    xt = jnp.transpose(A_q[0])
    kt = jnp.transpose(A_k[0])
    vt = jnp.transpose(A_v[0])
    sht = jnp.transpose(A_shift_k)
    wpt = jnp.transpose(B_w_phi, (1, 2, 0))
    out_t = pl.pallas_call(
        _kernel,
        grid=(NB + 4 - MERGE,),
        in_specs=[pl.BlockSpec(memory_space=pl.ANY)] * 10,
        out_specs=pl.BlockSpec(memory_space=pl.ANY),
        out_shape=jax.ShapeDtypeStruct((D, S), BF16),
        scratch_shapes=[
            pltpu.VMEM((NB, D, TS), BF16),
            pltpu.VMEM((D, S), BF16),
            pltpu.VMEM((D, S), BF16),
            pltpu.VMEM((D, S), BF16),
            pltpu.VMEM((4, D), BF16),
            pltpu.VMEM((D,), BF16),
            pltpu.VMEM((3, D, 3 * C), BF16),
            pltpu.VMEM((D, D), BF16),
            pltpu.VMEM((DH, DH, H), BF16),
            pltpu.VMEM((D, D), BF16),
            pltpu.VMEM((D,), BF16),
            pltpu.VMEM((2, 2, C // 2, C), U32),
            pltpu.VMEM((5, D, C), F32),
            pltpu.VMEM((DH, D), F32),
            pltpu.VMEM((KT, WROWS // 2, C), U32),
            pltpu.VMEM((KT, D // 2, C), U32),
            *[pltpu.VMEM((6, NCH, 16, C), F32) for _ in range(4)],
            pltpu.VMEM((NCH // 2, 2 * D, C), F32),
            pltpu.VMEM((NCH, NG, GR, C), U32),
            pltpu.VMEM((NG, NT_, GR, C), U32),
            pltpu.VMEM((NCH, 8, C), F32),
            pltpu.VMEM((NG, 80, C), F32),
            pltpu.VMEM((NG, 16, 80), F32),
            pltpu.VMEM((NCH, KT * C, C), BF16),
            pltpu.VMEM((4, 16, 2 * GR), F32),
            pltpu.VMEM((NG, 16, C), F32),
            pltpu.VMEM((NG, GR, C), F32),
            pltpu.VMEM((D, S), BF16),
            pltpu.SemaphoreType.DMA((9 + NB,)),
        ],
        compiler_params=pltpu.CompilerParams(
            dimension_semantics=("arbitrary",), vmem_limit_bytes=100 * 1024 * 1024),
    )(xt, kt, vt, sht, A_ssm_k, A_ssm_D, B_wqkv, wpt, B_wo, gate_w)
    return jnp.transpose(out_t)[None]
```

```python
import numpy as np
import jax
import jax.numpy as jnp
from jax import lax
import jax.experimental.pallas as pl
import jax.experimental.pallas.tpu as pltpu

S, D, H, DH = 2048, 576, 32, 18
C = 128
NCH = S // C
SKEW = 3
TS = 256
NT_ = TS // C
NB = S // TS
NG = 8
GR = 72
KT = 5
LOG2E = 1.4426950408889634
F32, BF16, U32 = jnp.float32, jnp.bfloat16, jnp.uint32

WK0, WQ0, WV0, WROWS = 0, 576, 1088, 1680

ORDER0 = "K0 K1 Q0 K2 Q1 K3 Q2 W Q3 V0 FH1 FU0 V1 KV0 FH0 FU1 V2 KV1 FH2 V3 KV2 FU2 KV3".split()
ORDER1 = ("K00 K10 V00 V10 Q10 Q00 KA0 LA0 IN0 FH0 FU0 KB0 LB0 K01 K11 V11 V01 Q11 Q01 KA1 LA1 KB1 IN1 LB1 FH1 FU1 "
          "K02 K12 V12 V02 Q12 Q02 KA2 LA2 IN2 KB2 LB2 FH2 FU2 K03 K13 V03 V13 Q13 FU3 Q03 KA3 LA3 KB3 LB3 FH3 IN3").split()
PACE = [{7: "K00"}, {1: "FH0", 8: "K11"}, {0: "IN1", 8: "K02", 12: "V02"}, {0: "FU2", 11: "sK03", 9: "FU2", 13: "sK03"}]
OLAG = 2
CPOS = (4, 8, 12, 17, 20, 32, 35, 48)
FOFF = (0, 1, 0, 3)
OBS = (0, 192, 384, 512, 576)
LSPLIT = (0, 10, 14, 16)
WCH = (0, 3, 6, 9)
PORDER = (0, 1, 4, 5, 8, 9, 12, 13)

NN = (((1,), (0,)), ((), ()))
NT = (((1,), (1,)), ((), ()))
TN = (((0,), (0,)), ((), ()))


def _dot(a, b, dims=NN):
    return lax.dot_general(a, b, dims, preferred_element_type=F32)


def _pk(x):
    return pltpu.bitcast(x.astype(BF16), U32)


def _up(x):
    return pltpu.bitcast(x, BF16)


def _iota(shape, dim):
    return lax.broadcasted_iota(jnp.int32, shape, dim)


def _tree(op, xs):
    xs = list(xs)
    while len(xs) > 1:
        nxt = [op(xs[i], xs[i + 1]) for i in range(0, len(xs) - 1, 2)]
        if len(xs) % 2:
            nxt.append(xs[-1])
        xs = nxt
    return xs[0]


def _softmax_pair(p, last):
    ps = [p[8 * j:8 * j + 8] for j in range(8)] + [last]
    mx = _tree(jnp.maximum, ps)
    mn = _tree(jnp.minimum, ps)
    mx = jnp.maximum(mx, pltpu.roll(mx, 4, 0))
    mn = jnp.minimum(mn, pltpu.roll(mn, 4, 0))
    ep = [jnp.exp2(x - mx) for x in ps]
    en = [jnp.exp2(mn - x) for x in ps]
    sp = _tree(jnp.add, ep)
    sn = _tree(jnp.add, en)
    rp = pl.reciprocal(sp + pltpu.roll(sp, 4, 0), approx=True)
    rn = pl.reciprocal(sn + pltpu.roll(sn, 4, 0), approx=True)
    out = []
    for a, b in zip(ep, en):
        out += [a * rp, b * rn]
    return jnp.concatenate(out, axis=0)


def _load_wide(ref, r0, r1, full=False):
    rows = slice(r0 // 2, r1 // 2)
    last = ref[KT - 1, rows, :] if full else ref[KT - 1, rows, 0:64]
    return _up(jnp.concatenate([ref[t, rows, :] for t in range(KT - 1)] + [last], axis=1))


def _store_wide(ref, r0, r1, val):
    rows = slice(r0 // 2, r1 // 2)
    w = _pk(val)
    for t in range(KT - 1):
        ref[t, rows, :] = w[:, t * C:(t + 1) * C]
    ref[KT - 1, rows, 0:64] = w[:, (KT - 1) * C:D]


def _kernel(x_hbm, k_hbm, v_hbm, sh_hbm, h_hbm, d_hbm, wqkv_hbm, wphi_hbm, wo_hbm, gw_hbm,
            o_hbm,
            x_v, k_v, v_v, h_v, sh_v, d_v, wqk_v, wv_v, wphi_v, wo_v, gw_v,
            f_v, col_v, wcat_v, wt_v, wot_v, ab0, ab1, ab2, ab3, y_v, phiq_v, phik_v,
            g_v, kv_v, kvl_v, ot_v, dp_v, zl_v, cb_v, o_v, rd_v, ok_v,
            sems):
    step = pl.program_id(0)
    ab_l = [ab0, ab1, ab2, ab3]
    never = _iota((8, C), 0) < -step
    glink = [None]
    sub = _iota((8, C), 0)

    def a_copies(sem, start, size):
        rows = pl.ds(start, size)
        return [pltpu.make_async_copy(src.at[rows], dst.at[rows], sems.at[sem])
                for src, dst in ((k_hbm, k_v), (v_hbm, v_v), (h_hbm, h_v))]

    def x_copy(sem, i):
        return pltpu.make_async_copy(x_hbm.at[:, pl.ds(i * TS, TS)], x_v.at[i], sems.at[sem])

    def wqk_copy(sem, c):
        cols = pl.ds(WCH[c] * C, (WCH[c + 1] - WCH[c]) * C)
        return pltpu.make_async_copy(wqkv_hbm.at[:, cols], wqk_v.at[:, cols], sems.at[sem])

    cp_phi = [pltpu.make_async_copy(wphi_hbm, wphi_v, sems.at[0])]
    cp_w0 = [wqk_copy(1, 0)]
    cp_w1 = [wqk_copy(2, 1)] + [pltpu.make_async_copy(src, dst, sems.at[2])
                                for src, dst in ((sh_hbm, sh_v), (d_hbm, d_v), (gw_hbm, gw_v))]
    cp_w2 = [wqk_copy(3, 2), x_copy(3, 0)]
    cp_w3 = [pltpu.make_async_copy(wqkv_hbm.at[:, pl.ds(2 * D, D)], wv_v, sems.at[4])] + a_copies(4, 0, 16 * SKEW)

    def cp_step(s):
        return [x_copy(4 + s, s)] + a_copies(4 + s, pl.multiple_of(16 * SKEW + (s - 1) * 64, 16), 64)

    a_done = 16 * SKEW + (NB - 1) * 64
    cp_last = a_copies(4 + NB, a_done, D - a_done) + [pltpu.make_async_copy(wo_hbm, wo_v, sems.at[4 + NB])]

    def out_copy(j, c0=0, c1=NCH, sem=None):
        rows = pl.ds(OBS[j], OBS[j + 1] - OBS[j])
        cols = pl.ds(c0 * C, (c1 - c0) * C)
        return pltpu.make_async_copy(o_v.at[rows, cols], o_hbm.at[rows, cols],
                                     sems.at[5 + NB + (j if sem is None else sem)])

    def wait(cps):
        for cp in cps:
            cp.wait()

    def fmat(e):
        return _up(jnp.concatenate([f_v[e, 0], f_v[e, 1]], axis=1))

    def a_fwd_h(n, ab):
        rows = pl.ds(pl.multiple_of(n * 16, 16), 16)
        hts = []
        for e in range(2):
            cs = [e + 2 * t for t in range(8)]
            hts.append(_dot(jnp.concatenate([h_v[rows, c * C:(c + 1) * C] for c in cs], axis=0), fmat(e)))
        for c in range(NCH):
            t = c // 2
            hc = hts[c % 2][t * 16:(t + 1) * 16, 0:C]
            hd = hts[c % 2][t * 16:(t + 1) * 16, C:2 * C]
            if c == 0:
                gcr, gd = hc + col_v[4, rows, :], hd
            elif c % 2:
                gcr, gd = hc + pc, hd + pd
            else:
                gcr, gd = hc - pc, hd - pd
            ab[3, c] = gcr
            ab[4, c] = gd - gcr
            ab[5, c] = gd + gcr
            pc, pd = hc, hd
        return hts[0][0:8, 0:C]

    def a_fwd_u(n, ab):
        rows = pl.ds(pl.multiple_of(n * 16, 16), 16)
        lane = _iota((16, C), 1)
        w = [col_v[j, rows, :] for j in range(4)]
        prev = [jnp.zeros((16, C), F32)] * 3
        us = []
        for c in range(NCH):
            kk = k_v[rows, c * C:(c + 1) * C].astype(F32)
            acc = kk * w[0]
            cur = []
            for j in range(1, 4):
                r = pltpu.roll(kk * w[j], j, 1)
                cur.append(r)
                acc = acc + jnp.where(lane < j, prev[j - 1], r)
            prev = cur
            us.append(acc * v_v[rows, c * C:(c + 1) * C].astype(F32))
        for e in range(2):
            cs = [e + 2 * t for t in range(8)]
            ft = _dot(jnp.concatenate([us[c] for c in cs], axis=0).astype(BF16), fmat(e))
            for t, c in enumerate(cs):
                a = ft[t * 16:(t + 1) * 16, 0:C]
                b = ft[t * 16:(t + 1) * 16, C:2 * C]
                ab[0, c] = a
                ab[1, c] = b
                ab[2, c] = a + b
        return ft[0:8, 0:C]

    def a_conv_inv(n, ab, gates=None):
        res = {}
        link = glink[0]
        for hf in range(2):
            pr = slice(8 * hf, 8 * hf + 8)

            def chain(o, gq, uq, acc, neg):
                for a in range(o + 1):
                    t = ab[gq, a, pr, :] * ab[uq, o - a, pr, :]
                    if acc is None:
                        acc = t if link is None else jnp.where(never, link, t)
                    elif bool((a & 1) and ((o - a) & 1)) != neg:
                        acc = acc - t
                    else:
                        acc = acc + t
                return acc

            for pi, o0 in enumerate(PORDER):
                os_ = (o0, o0 + 2)
                if gates and (8 * hf + pi) in gates:
                    tk = gates[8 * hf + pi]
                    link = tk if link is None else jnp.where(never, tk, link)
                k1 = [chain(o, 3, 2, None, False) for o in os_]
                re = [chain(o, 5, 1, k, True) for o, k in zip(os_, k1)]
                rep = _pk(jnp.concatenate(re, axis=0))
                link = pltpu.bitcast(rep, F32)
                k1 = [jnp.where(never, link, k) for k in k1]
                im = [chain(o, 4, 0, k, False) for o, k in zip(os_, k1)]
                imp = _pk(jnp.concatenate(im, axis=0))
                link = pltpu.bitcast(imp, F32)
                res[(o0, hf)] = (rep, imp)
        glink[0] = link
        for e in range(2):
            order = [(o0, hf) for hf in range(2) for o0 in PORDER if (o0 & 1) == e]
            lhs = _up(jnp.concatenate(
                [jnp.concatenate([res[k][0] for k in order], axis=0),
                 jnp.concatenate([res[k][1] for k in order], axis=0)], axis=1))
            yt = _dot(lhs, fmat(e), NT)
            for n_, (o0, hf) in enumerate(order):
                rows = pl.ds(pl.multiple_of(n * 16 + 8 * hf, 8), 8)
                y_v[o0, rows, :] = yt[16 * n_:16 * n_ + 8]
                y_v[o0 + 2, rows, :] = yt[16 * n_ + 8:16 * n_ + 16]
        return yt[0:8]

    def feat(p, shared):
        return [_softmax_pair(p[0:64], jnp.where(sub < 4, shared, 0.0)),
                _softmax_pair(p[64:128], jnp.where(sub < 4, 0.0, shared))]

    def proj(xs, r0, r1, t):
        return _dot(_load_wide(wt_v, r0, r1), xs[t])

    def k_unit(xs, r, t):
        p = proj(xs, WK0 + 144 * r, WK0 + 144 * (r + 1), t)
        return feat(p[16:144], p[0:8]), p[8:16]

    def q_unit(xs, i, r, t, sq):
        p = proj(xs, WQ0 + 128 * r, WQ0 + 128 * (r + 1), t)
        for e, ph in enumerate(feat(p, sq)):
            phiq_v[i * NT_ + t, 2 * r + e] = ph.astype(BF16)

    def v_unit(xs, i, r, t):
        p = proj(xs, WV0 + 144 * r, WV0 + 144 * (r + 1) + (16 if r == 3 else 0), t)
        if r == 3:
            g_v[i * NT_ + t] = jax.nn.sigmoid(p[2 * GR:2 * GR + 8])
        return p

    def kv_unit(g, pks, pvs, first=False, part=3):
        e = g % 2
        phik = jnp.concatenate(pks, axis=1)
        vb = jnp.concatenate(
            [jnp.concatenate([p[GR * e:GR * (e + 1)] for p in pvs], axis=1), jnp.ones((8, TS), F32)],
            axis=0).astype(BF16)
        if part & 1:
            a = _dot(vb, phik[0:C].astype(BF16), NT)
            kv_v[g] = a if first else kv_v[g] + a
        if part & 2:
            b = _dot(phik[C:2 * GR].astype(BF16), vb, NT)
            kvl_v[g] = b if first else kvl_v[g] + b

    def out_unit(j, ct):
        ra, rb_ = OBS[j], OBS[j + 1]
        gs = jnp.concatenate([g_v[ct] * (1.0 / C)] * 2, axis=0)
        bt = _dot(_load_wide(wot_v, ra, rb_, full=True), ot_v[ct])
        for r0 in range(ra, rb_, 16):
            y = y_v[ct, r0:r0 + 16, :]
            xq = x_v[ct // NT_, r0:r0 + 16, (ct % NT_) * C:(ct % NT_ + 1) * C].astype(F32)
            o_v[r0:r0 + 16, ct * C:(ct + 1) * C] = (bt[r0 - ra:r0 - ra + 16] + (xq * gs) * y).astype(BF16)

    @pl.when(step == 0)
    def _():
        for cp in cp_phi + cp_w0 + cp_w1 + cp_w2 + cp_w3:
            cp.start()
        for s in range(1, NB):
            for cp in cp_step(s):
                cp.start()
        for cp in cp_last:
            cp.start()

        n = _iota((24, C), 0)
        f = _iota((24, C), 1)
        n = jnp.where(n < 8, n, 8 * (n - 8))
        ang = (((2 * f + 1) * n) & 511).astype(F32) * (np.pi / 256)
        ct_, st_ = jnp.cos(ang), jnp.sin(ang)
        cs, sn = [], []
        for a in range(16):
            ca = jnp.broadcast_to(ct_[8 + a:9 + a], (8, C))
            sa = jnp.broadcast_to(st_[8 + a:9 + a], (8, C))
            cs.append(ca * ct_[0:8] - sa * st_[0:8])
            sn.append(sa * ct_[0:8] + ca * st_[0:8])
        cs, sn = jnp.concatenate(cs, axis=0), jnp.concatenate(sn, axis=0)
        sg = (1 - 2 * (_iota((C, C), 1) & 1)).astype(F32)
        f_v[0, 0] = _pk(cs)
        f_v[0, 1] = _pk(-sn)
        f_v[1, 0] = _pk(-sg * sn)
        f_v[1, 1] = _pk(-sg * cs)
        er = _iota((D, D), 0)
        ec = _iota((D, D), 1)
        perm = (ec == 18 * (er & 31) + (er >> 5)).astype(BF16)

        wait(cp_phi)
        for d in range(DH):
            wcat_v[:, 32 * d:32 * d + 32] = wphi_v[d].astype(F32)
        rep = (_iota((GR, DH), 0) // 4 == _iota((GR, DH), 1)).astype(BF16)
        whd = _dot(wcat_v[...].astype(BF16), perm).astype(BF16)
        t1 = _dot(rep, whd)
        t1 = jnp.concatenate([t1, t1], axis=1)

        rowg = _iota((GR, C), 0) & 3
        colc = _iota((GR, C), 1)
        lo4 = _iota((8, D), 0) < 4
        parts, d16 = {}, {}

        def fold(t):
            gs = [g for g in range(2 * NG) if GR * g < C * (t + 1) and GR * (g + 1) > C * t]
            tile = t1[:, t * C:(t + 1) * C]
            lhs = []
            for g in gs:
                lo = 18 * rowg + (GR * g - C * t)
                lhs.append(jnp.where((colc >= lo) & (colc < lo + 18), tile, 0.0))
            lhs = jnp.concatenate(lhs, axis=0).astype(BF16)
            res = _dot(lhs, wqk_v[:, t * C:(t + 1) * C], NT)
            for n_, g in enumerate(gs):
                piece = res[n_ * GR:(n_ + 1) * GR]
                parts[g] = piece if g not in parts else parts[g] + piece
                if GR * (g + 1) <= C * (t + 1):
                    w = parts[g] * LOG2E
                    tail = w[64:72]
                    swap = pltpu.roll(tail, 4, 0)
                    w17 = jnp.where(lo4, swap, tail)
                    main = jnp.concatenate([w[8 * j:8 * j + 8] - w17 for j in range(8)], axis=0)
                    d16[g] = (tail - swap) if g % 2 == 0 else (swap - tail)
                    if g < NG:
                        r0 = WQ0 + 64 * g
                    else:
                        r0 = WK0 + 144 * ((g - NG) // 2) + 16 + 64 * (g % 2)
                    _store_wide(wt_v, r0, r0 + 64, main)
                    if g >= NG and g % 2 == 1:
                        r0 = WK0 + 144 * ((g - NG) // 2)
                        _store_wide(wt_v, r0, r0 + 16, jnp.concatenate(
                            [jnp.where(lo4, d16[g - 1], d16[g]), jnp.where(lo4, d16[g - 1 - NG], d16[g - NG])],
                            axis=0))

        wait(cp_w0)
        for t in range(WCH[0], WCH[1]):
            fold(t)
        wait(cp_w1)
        for t in range(WCH[1], WCH[2]):
            fold(t)
        _store_wide(wt_v, WV0 + D, WROWS, jnp.broadcast_to(gw_v[...].reshape(1, D).astype(F32), (16, D)))
        wait(cp_w2)
        for t in range(WCH[2], WCH[3]):
            fold(t)
        sh = sh_v[...].astype(F32)
        for j in range(5):
            row = sh[j:j + 1, :] if j < 4 else d_v[...].reshape(1, D).astype(F32)
            col_v[j] = jnp.broadcast_to(row, (C, D)).T
        xs = [x_v[0, :, t * C:(t + 1) * C] for t in range(NT_)]
        sq, pv = {}, {}
        for u in ORDER0:
            if u == "W":
                wait(cp_w3)
                _store_wide(wt_v, WV0, WV0 + D, wv_v[...].T)
                xs = [x_v[0, :, t * C:(t + 1) * C] for t in range(NT_)]
                continue
            op, r = u[:-1], int(u[-1])
            if op == "K":
                for t in range(NT_):
                    pk, sq[r, t] = k_unit(xs, r, t)
                    for e in range(2):
                        phik_v[2 * r + e, t] = pk[e].astype(BF16)
            elif op == "Q":
                for t in range(NT_):
                    q_unit(xs, 0, r, t, sq[r, t])
            elif op == "V":
                pv[r] = [v_unit(xs, 0, r, t) for t in range(NT_)]
            elif op == "KV":
                for g in (2 * r, 2 * r + 1):
                    kv_unit(g, [phik_v[g, t] for t in range(NT_)], pv[r], first=True)
            elif op == "FH":
                a_fwd_h(r, ab_l[r])
            elif op == "FU":
                a_fwd_u(r, ab_l[r])

    @pl.when((step >= 1) & (step < NB))
    def _():
        i = step
        wait(cp_step(step))
        glink[0] = None
        xs = [x_v[i, :, t * C:(t + 1) * C] for t in range(NT_)]
        n0 = 4 * (step - 1)
        pk, pv, sq, toks = {}, {}, {}, {}
        for u in ORDER1:
            op, r = u[:2], int(u[2])
            if op in ("K0", "K1"):
                t = int(op[1])
                pk[r, t], sq[r, t] = k_unit(xs, r, t)
                toks[u] = sq[r, t]
                toks["s" + u] = pk[r, t][1][136:144]
            elif op in ("V0", "V1"):
                pv[r, int(op[1])] = v_unit(xs, i, r, int(op[1]))
                toks[u] = pv[r, int(op[1])][0:8]
            elif op in ("Q0", "Q1"):
                q_unit(xs, i, r, int(op[1]), sq[r, int(op[1])])
            elif op in ("KA", "KB", "LA", "LB"):
                e = 0 if op[1] == "A" else 1
                kv_unit(2 * r + e, [pk[r, t][e] for t in range(NT_)], [pv[r, t] for t in range(NT_)],
                        part=1 if op[0] == "K" else 2)
            elif op == "FH":
                toks[u] = a_fwd_h(n0 + r + SKEW, ab_l[(r + SKEW) % 4])
            elif op == "FU":
                toks[u] = a_fwd_u(n0 + r + SKEW, ab_l[(r + SKEW) % 4])
            elif op == "IN":
                toks[u] = a_conv_inv(n0 + r, ab_l[r], {k: toks[v] for k, v in PACE[r].items()})
        zls = [kvl_v[g, :, GR:GR + 1] for g in range(NG)]
        zmin = jnp.minimum(jnp.min(_tree(jnp.minimum, [kv_v[g, GR:GR + 1, :] for g in range(NG)]), keepdims=True),
                           jnp.min(_tree(jnp.minimum, zls), keepdims=True))
        zmax = jnp.max(_tree(jnp.maximum, zls), keepdims=True)
        ok_v[...] = jnp.broadcast_to(jnp.where(zmax <= 4.0 * zmin, 1.0, 0.0), (16, C))

    N2 = 4 * (NB - 1)

    @pl.when(step == NB)
    def _():
        wait(cp_last)
        glink[0] = None

        def head_of(v):
            return (v >= 18).astype(jnp.int32) + (v >= 36).astype(jnp.int32) + (v >= 54).astype(jnp.int32)

        r = _iota((80, C), 0)
        hr = jnp.where(r < GR, head_of(r), r & 3)
        mmask = hr == (_iota((80, C), 1) & 3)
        ll, lr = _iota((16, 80), 1), _iota((16, 80), 0)
        lmask = (head_of(ll) == (lr & 3)) & (ll < GR)
        hi4 = (lr & 4) != 0
        is17 = [lmask & hi4, lmask & jnp.logical_not(hi4)]
        sel = (((_iota((16, C), 1) >> 3) & 1) == (_iota((16, C), 0) >> 3)).astype(BF16)
        slow = ok_v[0, 0] < 0.5
        fast = ok_v[:, 0:80] > 0.5
        a_fwd_h(N2 + SKEW, ab_l[SKEW % 4])
        kvm = []
        for g in range(NG):
            kvl = kvl_v[g]
            k17 = jnp.where(is17[g % 2] & fast, kvl, 0.0).astype(BF16)
            tt = _dot(k17, sel, TN)
            kvm.append(jnp.where(mmask, kv_v[g] - tt, 0.0).astype(BF16))
            cb_v[g] = tt[0:GR] + pltpu.roll(tt[0:GR], 8, 1)
            k17f = jnp.where(is17[g % 2] & fast, kvl, 0.0).astype(BF16).astype(F32)
            k17f = jnp.concatenate([pltpu.roll(k17f[0:8], 4, 0), pltpu.roll(k17f[8:16], 4, 0)], axis=0)
            dd = jnp.where(is17[1 - g % 2], kvl - k17f, 0.0)
            dp_v[g // 2, :, GR * (g % 2):GR * (g % 2) + GR] = dd[:, 0:GR]
            zl_v[g] = jnp.broadcast_to(kvl[:, GR:GR + 1], (16, C))
        m16 = [_dot(dp_v[r_].astype(BF16), wo_v[144 * r_:144 * (r_ + 1), :]) for r_ in range(4)]
        a_fwd_u(N2 + SKEW, ab_l[SKEW % 4])
        wlast = jnp.concatenate([wo_v[4 * C:D, :].astype(F32)] + m16, axis=0)
        wot_v[KT - 1] = _pk(wlast.T)
        w4 = pltpu.bitcast(wo_v[0:4 * C, :].T, U32)
        for t in range(KT - 1):
            wot_v[t] = w4[:, t * C:(t + 1) * C]

        def num_unit(ct):
            omg = 1.0 - g_v[ct]
            for gp in range(NG // 2):
                os_, xs_ = [], []
                for e in range(2):
                    g = 2 * gp + e
                    nd = _dot(kvm[g], phiq_v[ct, g, 0:C, :])
                    pl_ = phiq_v[ct, g, C:2 * GR, :].astype(F32)
                    ph = [pl_[0:8], pl_[8:16]]
                    dl = ph[0] * zl_v[g, 0:8, :] + ph[1] * zl_v[g, 8:16, :]
                    den = nd[GR:GR + 8] + (dl + pltpu.roll(dl, 4, 0)) + 1e-6
                    rd = omg * pl.reciprocal(den, approx=True)
                    rd_v[ct, g] = rd
                    b = [jnp.broadcast_to(rd[j:j + 1], (8, C)) for j in range(4)]
                    pat = [b[0], b[0], jnp.where(sub < 2, b[0], b[1]), b[1], jnp.where(sub < 4, b[1], b[2]), b[2],
                           jnp.where(sub < 6, b[2], b[3]), b[3], b[3]]
                    os_ += [(nd[8 * j:8 * j + 8] + cb_v[g, 8 * j:8 * j + 8, :]) * pat[j] for j in range(9)]
                    xs_.append((ph, rd))
                ot_v[ct, 2 * GR * gp:2 * GR * (gp + 1), :] = jnp.concatenate(os_, axis=0).astype(BF16)
                rd = jnp.where(sub < 4, xs_[0][1], xs_[1][1])
                xx = [jnp.where(sub < 4, xs_[0][0][sg_], xs_[1][0][sg_]) * rd for sg_ in range(2)]
                ot_v[ct, D + 16 * gp:D + 16 * (gp + 1), :] = jnp.concatenate(xx, axis=0).astype(BF16)

        nstep = NCH + OLAG
        for it in range(nstep + 2 * NCH):
            if it < NCH:
                num_unit(it)
            if OLAG <= it < nstep:
                out_unit(0, it - OLAG)
            elif it >= nstep:
                out_unit(1 + (it - nstep) // NCH, (it - nstep) % NCH)
            if it >= nstep - 1 and (it - nstep + 1) % NCH == 0:
                out_copy((it - nstep + 1) // NCH).start()
            for n_ in range(8):
                if it == CPOS[n_]:
                    a_conv_inv(N2 + n_, ab_l[n_ % 4])
                if n_ < 4 and it == CPOS[n_] + FOFF[n_]:
                    a_fwd_h(N2 + n_ + 4, ab_l[n_ % 4])
                    a_fwd_u(N2 + n_ + 4, ab_l[n_ % 4])
        last = [out_copy(3, a, b, 3 + n_) for n_, (a, b) in enumerate(zip(LSPLIT[:-1], LSPLIT[1:]))]
        for ct in range(NCH):
            out_unit(3, ct)
            if ct + 1 in LSPLIT:
                last[LSPLIT.index(ct + 1) - 1].start()
        wait([out_copy(j) for j in range(3)] + last)

        @pl.when(slow)
        def _():
            for g in range(NG):
                dp_v[g // 2, :, GR * (g % 2):GR * (g % 2) + GR] = jnp.where(is17[g % 2], kvl_v[g], 0.0)[:, 0:GR]
            m17 = jnp.concatenate(
                [_dot(dp_v[r_].astype(BF16), wo_v[144 * r_:144 * (r_ + 1), :]) for r_ in range(4)],
                axis=0).astype(BF16)

            def body(ct, carry):
                xs_ = []
                for gp in range(NG // 2):
                    pa = phiq_v[ct, 2 * gp, C:2 * GR, :].astype(F32)
                    pb = phiq_v[ct, 2 * gp + 1, C:2 * GR, :].astype(F32)
                    rd = jnp.where(sub < 4, rd_v[ct, 2 * gp + 1], rd_v[ct, 2 * gp])
                    xs_ += [jnp.where(sub < 4, pb[8 * sg_:8 * sg_ + 8], pa[8 * sg_:8 * sg_ + 8]) * rd
                            for sg_ in range(2)]
                corr = _dot(m17, jnp.concatenate(xs_, axis=0).astype(BF16), TN)
                cols = pl.ds(pl.multiple_of(ct * C, C), C)
                o_v[:, cols] = (o_v[:, cols].astype(F32) + corr).astype(BF16)
                return carry

            lax.fori_loop(0, NCH, body, 0)
            again = pltpu.make_async_copy(o_v, o_hbm, sems.at[5 + NB])
            again.start()
            again.wait()


@jax.jit
def pallas_gated_mix__ssm_conv_h3__linear_kernel_hedgehog__prompt_kernel(A_q, A_k, A_v, A_shift_k, A_ssm_k, A_ssm_D, B_x, B_wqkv, B_w_phi, B_wo, gate_w):
    del B_x
    xt = jnp.transpose(A_q[0])
    kt = jnp.transpose(A_k[0])
    vt = jnp.transpose(A_v[0])
    sht = jnp.transpose(A_shift_k)
    wpt = jnp.transpose(B_w_phi, (1, 2, 0))
    out_t = pl.pallas_call(
        _kernel,
        grid=(NB + 1,),
        in_specs=[pl.BlockSpec(memory_space=pl.ANY)] * 10,
        out_specs=pl.BlockSpec(memory_space=pl.ANY),
        out_shape=jax.ShapeDtypeStruct((D, S), BF16),
        scratch_shapes=[
            pltpu.VMEM((NB, D, TS), BF16),
            pltpu.VMEM((D, S), BF16),
            pltpu.VMEM((D, S), BF16),
            pltpu.VMEM((D, S), BF16),
            pltpu.VMEM((4, D), BF16),
            pltpu.VMEM((D,), BF16),
            pltpu.VMEM((D, 9 * C), BF16),
            pltpu.VMEM((D, D), BF16),
            pltpu.VMEM((DH, DH, H), BF16),
            pltpu.VMEM((D, D), BF16),
            pltpu.VMEM((D,), BF16),
            pltpu.VMEM((2, 2, C // 2, C), U32),
            pltpu.VMEM((5, D, C), F32),
            pltpu.VMEM((DH, D), F32),
            pltpu.VMEM((KT, WROWS // 2, C), U32),
            pltpu.VMEM((KT, D // 2, C), U32),
            *[pltpu.VMEM((6, NCH, 16, C), F32) for _ in range(4)],
            pltpu.VMEM((NCH, D, C), F32),
            pltpu.VMEM((NCH, NG, 2 * GR, C), BF16),
            pltpu.VMEM((NG, NT_, 2 * GR, C), BF16),
            pltpu.VMEM((NCH, 8, C), F32),
            pltpu.VMEM((NG, 80, C), F32),
            pltpu.VMEM((NG, 16, 80), F32),
            pltpu.VMEM((NCH, KT * C, C), BF16),
            pltpu.VMEM((4, 16, 2 * GR), F32),
            pltpu.VMEM((NG, 16, C), F32),
            pltpu.VMEM((NG, GR, C), F32),
            pltpu.VMEM((D, S), BF16),
            pltpu.VMEM((NCH, NG, 8, C), F32),
            pltpu.VMEM((16, C), F32),
            pltpu.SemaphoreType.DMA((7 + NB + len(LSPLIT),)),
        ],
        compiler_params=pltpu.CompilerParams(
            dimension_semantics=("arbitrary",), vmem_limit_bytes=100 * 1024 * 1024,
            disable_semaphore_checks=True),
    )(xt, kt, vt, sht, A_ssm_k, A_ssm_D, B_wqkv, wpt, B_wo, gate_w)
    return jnp.transpose(out_t)[None]
```

```python
import numpy as np
import jax
import jax.numpy as jnp
from jax import lax
import jax.experimental.pallas as pl
import jax.experimental.pallas.tpu as pltpu

S, D, H, DH = 2048, 576, 32, 18
C = 128
NCH = S // C
SKEW = 3
TS = 256
NT_ = TS // C
NB = S // TS
NG = 8
GR = 72
KT = 5
LOG2E = 1.4426950408889634
F32, BF16, U32 = jnp.float32, jnp.bfloat16, jnp.uint32

WK0, WQ0, WV0, WROWS = 0, 576, 1088, 1680

ORDER0 = "K0 K1 Q0 K2 Q1 K3 Q2 W Q3 V0 FH1 FU0 V1 KV0 FH0 FU1 V2 KV1 FH2 V3 KV2 FU2 KV3".split()
ORDER1 = ("K00 K10 V00 V10 Q10 Q00 KA0 LA0 IN0 FH0 FU0 KB0 LB0 K01 K11 V11 V01 Q11 Q01 KA1 LA1 KB1 IN1 LB1 FH1 FU1 "
          "K02 K12 V12 V02 Q12 Q02 KA2 LA2 IN2 KB2 LB2 FH2 FU2 K03 K13 V03 V13 Q13 FU3 Q03 KA3 LA3 KB3 LB3 FH3 IN3").split()
PACE = [{7: 'K00'}, {1: 'FH0', 8: 'K11'}, {0: 'IN1', 8: 'K02', 12: 'V02'}, {0: 'FU2', 11: 'sK03', 13: 'sK03', 9: 'Q13'}]
OLAG = 2
CPOS = (4, 8, 12, 17, 20, 28, 35, 48)
FOFF = (0, 1, 0, 3)
OBS = (0, 192, 384, 512, 576)
LSPLIT = (0, 10, 14, 16)
WCH = (0, 3, 6, 9)
PORDER = (0, 1, 4, 5, 8, 9, 12, 13)

PSEQ = ((0, 1, 2, 3, 4, 5, 6, 7, 8, 9, 10, 11, 13, 12, 14, 15),
        (0, 1, 2, 3, 4, 5, 6, 7, 8, 9, 10, 11, 13, 12, 14, 15),
        (0, 1, 3, 4, 5, 6, 7, 8, 2, 9, 10, 13, 11, 12, 14, 15),
        (0, 1, 2, 4, 5, 3, 6, 7, 8, 9, 10, 11, 12, 13, 14, 15))

NN = (((1,), (0,)), ((), ()))
NT = (((1,), (1,)), ((), ()))
TN = (((0,), (0,)), ((), ()))


def _dot(a, b, dims=NN):
    return lax.dot_general(a, b, dims, preferred_element_type=F32)


def _pk(x):
    return pltpu.bitcast(x.astype(BF16), U32)


def _up(x):
    return pltpu.bitcast(x, BF16)


def _iota(shape, dim):
    return lax.broadcasted_iota(jnp.int32, shape, dim)


def _tree(op, xs):
    xs = list(xs)
    while len(xs) > 1:
        nxt = [op(xs[i], xs[i + 1]) for i in range(0, len(xs) - 1, 2)]
        if len(xs) % 2:
            nxt.append(xs[-1])
        xs = nxt
    return xs[0]


def _softmax_pair(p, last):
    ps = [p[8 * j:8 * j + 8] for j in range(8)] + [last]
    mx = _tree(jnp.maximum, ps)
    mn = _tree(jnp.minimum, ps)
    mx = jnp.maximum(mx, pltpu.roll(mx, 4, 0))
    mn = jnp.minimum(mn, pltpu.roll(mn, 4, 0))
    ep = [jnp.exp2(x - mx) for x in ps]
    en = [jnp.exp2(mn - x) for x in ps]
    sp = _tree(jnp.add, ep)
    sn = _tree(jnp.add, en)
    rp = pl.reciprocal(sp + pltpu.roll(sp, 4, 0), approx=True)
    rn = pl.reciprocal(sn + pltpu.roll(sn, 4, 0), approx=True)
    out = []
    for a, b in zip(ep, en):
        out += [a * rp, b * rn]
    return jnp.concatenate(out, axis=0)


def _load_wide(ref, r0, r1, full=False):
    rows = slice(r0 // 2, r1 // 2)
    last = ref[KT - 1, rows, :] if full else ref[KT - 1, rows, 0:64]
    return _up(jnp.concatenate([ref[t, rows, :] for t in range(KT - 1)] + [last], axis=1))


def _store_wide(ref, r0, r1, val):
    rows = slice(r0 // 2, r1 // 2)
    w = _pk(val)
    for t in range(KT - 1):
        ref[t, rows, :] = w[:, t * C:(t + 1) * C]
    ref[KT - 1, rows, 0:64] = w[:, (KT - 1) * C:D]


def _kernel(x_hbm, k_hbm, v_hbm, sh_hbm, h_hbm, d_hbm, wqkv_hbm, wphi_hbm, wo_hbm, gw_hbm,
            o_hbm,
            x_v, k_v, v_v, h_v, sh_v, d_v, wqk_v, wv_v, wphi_v, wo_v, gw_v,
            f_v, col_v, wcat_v, wt_v, wot_v, ab0, ab1, ab2, ab3, y_v, phiq_v, phik_v,
            g_v, kv_v, kvl_v, ot_v, dp_v, zl_v, cb_v, o_v, rd_v, ok_v,
            sems):
    step = pl.program_id(0)
    ab_l = [ab0, ab1, ab2, ab3]
    never = _iota((8, C), 0) < -step
    glink = [None]
    sub = _iota((8, C), 0)
    lt2, lt4, lt6 = sub < 2, sub < 4, sub < 6

    def a_copies(sem, start, size):
        rows = pl.ds(start, size)
        return [pltpu.make_async_copy(src.at[rows], dst.at[rows], sems.at[sem])
                for src, dst in ((k_hbm, k_v), (v_hbm, v_v), (h_hbm, h_v))]

    def x_copy(sem, i):
        return pltpu.make_async_copy(x_hbm.at[:, pl.ds(i * TS, TS)], x_v.at[i], sems.at[sem])

    def wqk_copy(sem, c):
        cols = pl.ds(WCH[c] * C, (WCH[c + 1] - WCH[c]) * C)
        return pltpu.make_async_copy(wqkv_hbm.at[:, cols], wqk_v.at[:, cols], sems.at[sem])

    cp_phi = [pltpu.make_async_copy(wphi_hbm, wphi_v, sems.at[0])]
    cp_w0 = [wqk_copy(1, 0)]
    cp_w1 = [wqk_copy(2, 1)] + [pltpu.make_async_copy(src, dst, sems.at[2])
                                for src, dst in ((sh_hbm, sh_v), (d_hbm, d_v), (gw_hbm, gw_v))]
    cp_w2 = [wqk_copy(3, 2), x_copy(3, 0)]
    cp_w3 = [pltpu.make_async_copy(wqkv_hbm.at[:, pl.ds(2 * D, D)], wv_v, sems.at[4])] + a_copies(4, 0, 16 * SKEW)

    def cp_step(s):
        return [x_copy(s - 1, s)] + a_copies(s - 1, pl.multiple_of(16 * SKEW + (s - 1) * 64, 16), 64)

    a_done = 16 * SKEW + (NB - 1) * 64
    cp_last = a_copies(NB - 1, a_done, D - a_done) + [pltpu.make_async_copy(wo_hbm, wo_v, sems.at[NB - 1])]

    def out_copy(j, c0=0, c1=NCH, sem=None):
        rows = pl.ds(OBS[j], OBS[j + 1] - OBS[j])
        cols = pl.ds(c0 * C, (c1 - c0) * C)
        return pltpu.make_async_copy(o_v.at[rows, cols], o_hbm.at[rows, cols],
                                     sems.at[j if sem is None else sem])

    def wait(cps):
        for cp in cps:
            cp.wait()

    def start(cps):
        for cp in cps:
            cp.start()

    def fmat(e):
        return _up(jnp.concatenate([f_v[e, 0], f_v[e, 1]], axis=1))

    def a_fwd_h(n, ab):
        rows = pl.ds(pl.multiple_of(n * 16, 16), 16)
        hts = []
        for e in range(2):
            cs = [e + 2 * t for t in range(8)]
            hts.append(_dot(jnp.concatenate([h_v[rows, c * C:(c + 1) * C] for c in cs], axis=0), fmat(e)))
        for c in range(NCH):
            t = c // 2
            hc = hts[c % 2][t * 16:(t + 1) * 16, 0:C]
            hd = hts[c % 2][t * 16:(t + 1) * 16, C:2 * C]
            if c == 0:
                gcr, gd = hc + col_v[4, rows, :], hd
            elif c % 2:
                gcr, gd = hc + pc, hd + pd
            else:
                gcr, gd = hc - pc, hd - pd
            ab[3, c] = gcr
            ab[4, c] = gd - gcr
            ab[5, c] = gd + gcr
            pc, pd = hc, hd
        return hts[0][0:8, 0:C]

    def a_fwd_u(n, ab):
        rows = pl.ds(pl.multiple_of(n * 16, 16), 16)
        lane = _iota((16, C), 1)
        wrap = [lane < j for j in range(4)]
        w = [col_v[j, rows, :] for j in range(4)]
        prev = [jnp.zeros((16, C), F32)] * 3
        us = []
        for c in range(NCH):
            kk = k_v[rows, c * C:(c + 1) * C].astype(F32)
            acc = kk * w[0]
            cur = []
            for j in range(1, 4):
                r = pltpu.roll(kk * w[j], j, 1)
                cur.append(r)
                acc = acc + jnp.where(wrap[j], prev[j - 1], r)
            prev = cur
            us.append(acc * v_v[rows, c * C:(c + 1) * C].astype(F32))
        for e in range(2):
            cs = [e + 2 * t for t in range(8)]
            ft = _dot(jnp.concatenate([us[c] for c in cs], axis=0).astype(BF16), fmat(e))
            for t, c in enumerate(cs):
                a = ft[t * 16:(t + 1) * 16, 0:C]
                b = ft[t * 16:(t + 1) * 16, C:2 * C]
                ab[0, c] = a
                ab[1, c] = b
                ab[2, c] = a + b
        return ft[0:8, 0:C]

    def a_conv_inv(n, ab, gates=None, seq=None):
        res = {}
        link = glink[0]
        seq = [(v // 8, PORDER[v % 8]) for v in (seq or range(16))]

        loaded = {}

        def ld(q, c, hf):
            if (q, c, hf) not in loaded:
                loaded[q, c, hf] = ab[q, c, 8 * hf:8 * hf + 8, :]
            return loaded[q, c, hf]

        def chain(hf, o, gq, uq, acc, neg):
            for a in range(o + 1):
                t = ld(gq, a, hf) * ld(uq, o - a, hf)
                if acc is None:
                    acc = t if link is None else jnp.where(never, link, t)
                elif bool((a & 1) and ((o - a) & 1)) != neg:
                    acc = acc - t
                else:
                    acc = acc + t
            return acc

        for pi, (hf, o0) in enumerate(seq):
            os_ = (o0, o0 + 2)
            if gates and pi in gates:
                tk = gates[pi]
                link = tk if link is None else jnp.where(never, tk, link)
            k1 = [chain(hf, o, 3, 2, None, False) for o in os_]
            re = [chain(hf, o, 5, 1, k, True) for o, k in zip(os_, k1)]
            rep = _pk(jnp.concatenate(re, axis=0))
            link = pltpu.bitcast(rep, F32)
            k1 = [jnp.where(never, link, k) for k in k1]
            im = [chain(hf, o, 4, 0, k, False) for o, k in zip(os_, k1)]
            imp = _pk(jnp.concatenate(im, axis=0))
            link = pltpu.bitcast(imp, F32)
            res[(o0, hf)] = (rep, imp)
        glink[0] = link
        for e in range(2):
            order = [(o0, hf) for hf, o0 in seq if (o0 & 1) == e]
            lhs = _up(jnp.concatenate(
                [jnp.concatenate([res[k][0] for k in order], axis=0),
                 jnp.concatenate([res[k][1] for k in order], axis=0)], axis=1))
            yt = _dot(lhs, fmat(e), NT)
            for n_, (o0, hf) in enumerate(order):
                rows = pl.ds(pl.multiple_of(n * 16 + 8 * hf, 8), 8)
                y_v[o0, rows, :] = yt[16 * n_:16 * n_ + 8]
                y_v[o0 + 2, rows, :] = yt[16 * n_ + 8:16 * n_ + 16]
        return yt[0:8]

    def feat(p, shared):
        return [_softmax_pair(p[0:64], jnp.where(lt4, shared, 0.0)),
                _softmax_pair(p[64:128], jnp.where(lt4, 0.0, shared))]

    def proj(xs, r0, r1, t):
        return _dot(_load_wide(wt_v, r0, r1), xs[t])

    def k_unit(xs, r, t):
        p = proj(xs, WK0 + 144 * r, WK0 + 144 * (r + 1), t)
        return feat(p[16:144], p[0:8]), p[8:16]

    def q_unit(xs, i, r, t, sq):
        p = proj(xs, WQ0 + 128 * r, WQ0 + 128 * (r + 1), t)
        for e, ph in enumerate(feat(p, sq)):
            phiq_v[i * NT_ + t, 2 * r + e] = ph.astype(BF16)
        return p[0:8]

    def v_unit(xs, i, r, t):
        p = proj(xs, WV0 + 144 * r, WV0 + 144 * (r + 1) + (16 if r == 3 else 0), t)
        if r == 3:
            g_v[i * NT_ + t] = jax.nn.sigmoid(p[2 * GR:2 * GR + 8])
        return p

    def kv_unit(g, pks, pvs, first=False, part=3):
        e = g % 2
        phik = jnp.concatenate(pks, axis=1)
        vb = jnp.concatenate(
            [jnp.concatenate([p[GR * e:GR * (e + 1)] for p in pvs], axis=1), jnp.ones((8, TS), F32)],
            axis=0).astype(BF16)
        if part & 1:
            a = _dot(vb, phik[0:C].astype(BF16), NT)
            kv_v[g] = a if first else kv_v[g] + a
        if part & 2:
            b = _dot(phik[C:2 * GR].astype(BF16), vb, NT)
            kvl_v[g] = b if first else kvl_v[g] + b

    def out_unit(j, ct):
        ra, rb_ = OBS[j], OBS[j + 1]
        gs = jnp.concatenate([g_v[ct] * (1.0 / C)] * 2, axis=0)
        bt = _dot(_load_wide(wot_v, ra, rb_, full=True), ot_v[ct])
        for r0 in range(ra, rb_, 16):
            y = y_v[ct, r0:r0 + 16, :]
            xq = x_v[ct // NT_, r0:r0 + 16, (ct % NT_) * C:(ct % NT_ + 1) * C].astype(F32)
            o_v[r0:r0 + 16, ct * C:(ct + 1) * C] = (bt[r0 - ra:r0 - ra + 16] + (xq * gs) * y).astype(BF16)

    @pl.when(step == 0)
    def _():
        start(cp_phi + cp_w0 + cp_w1 + cp_w2 + cp_w3)

        n = _iota((24, C), 0)
        f = _iota((24, C), 1)
        n = jnp.where(n < 8, n, 8 * (n - 8))
        ang = (((2 * f + 1) * n) & 511).astype(F32) * (np.pi / 256)
        ct_, st_ = jnp.cos(ang), jnp.sin(ang)
        cs, sn = [], []
        for a in range(16):
            ca = jnp.broadcast_to(ct_[8 + a:9 + a], (8, C))
            sa = jnp.broadcast_to(st_[8 + a:9 + a], (8, C))
            cs.append(ca * ct_[0:8] - sa * st_[0:8])
            sn.append(sa * ct_[0:8] + ca * st_[0:8])
        cs, sn = jnp.concatenate(cs, axis=0), jnp.concatenate(sn, axis=0)
        sg = (1 - 2 * (_iota((C, C), 1) & 1)).astype(F32)
        f_v[0, 0] = _pk(cs)
        f_v[0, 1] = _pk(-sn)
        f_v[1, 0] = _pk(-sg * sn)
        f_v[1, 1] = _pk(-sg * cs)
        er = _iota((D, D), 0)
        ec = _iota((D, D), 1)
        perm = (ec == 18 * (er & 31) + (er >> 5)).astype(BF16)

        wait(cp_phi)
        start(cp_step(1))
        for d in range(DH):
            wcat_v[:, 32 * d:32 * d + 32] = wphi_v[d].astype(F32)
        rep = (_iota((GR, DH), 0) // 4 == _iota((GR, DH), 1)).astype(BF16)
        whd = _dot(wcat_v[...].astype(BF16), perm).astype(BF16)
        t1 = _dot(rep, whd)
        t1 = jnp.concatenate([t1, t1], axis=1)

        rowg = _iota((GR, C), 0) & 3
        colc = _iota((GR, C), 1)
        lo4 = _iota((8, D), 0) < 4
        parts, d16 = {}, {}

        def fold(t):
            gs = [g for g in range(2 * NG) if GR * g < C * (t + 1) and GR * (g + 1) > C * t]
            tile = t1[:, t * C:(t + 1) * C]
            lhs = []
            for g in gs:
                lo = 18 * rowg + (GR * g - C * t)
                lhs.append(jnp.where((colc >= lo) & (colc < lo + 18), tile, 0.0))
            lhs = jnp.concatenate(lhs, axis=0).astype(BF16)
            res = _dot(lhs, wqk_v[:, t * C:(t + 1) * C], NT)
            for n_, g in enumerate(gs):
                piece = res[n_ * GR:(n_ + 1) * GR]
                parts[g] = piece if g not in parts else parts[g] + piece
                if GR * (g + 1) <= C * (t + 1):
                    w = parts[g] * LOG2E
                    tail = w[64:72]
                    swap = pltpu.roll(tail, 4, 0)
                    w17 = jnp.where(lo4, swap, tail)
                    main = jnp.concatenate([w[8 * j:8 * j + 8] - w17 for j in range(8)], axis=0)
                    d16[g] = (tail - swap) if g % 2 == 0 else (swap - tail)
                    if g < NG:
                        r0 = WQ0 + 64 * g
                    else:
                        r0 = WK0 + 144 * ((g - NG) // 2) + 16 + 64 * (g % 2)
                    _store_wide(wt_v, r0, r0 + 64, main)
                    if g >= NG and g % 2 == 1:
                        r0 = WK0 + 144 * ((g - NG) // 2)
                        _store_wide(wt_v, r0, r0 + 16, jnp.concatenate(
                            [jnp.where(lo4, d16[g - 1], d16[g]), jnp.where(lo4, d16[g - 1 - NG], d16[g - NG])],
                            axis=0))

        wait(cp_w0)
        start(cp_step(2))
        for t in range(WCH[0], WCH[1]):
            fold(t)
        wait(cp_w1)
        start(cp_step(3))
        for t in range(WCH[1], WCH[2]):
            fold(t)
        _store_wide(wt_v, WV0 + D, WROWS, jnp.broadcast_to(gw_v[...].reshape(1, D).astype(F32), (16, D)))
        wait(cp_w2)
        start(cp_step(4))
        for t in range(WCH[2], WCH[3]):
            fold(t)
        sh = sh_v[...].astype(F32)
        for j in range(5):
            row = sh[j:j + 1, :] if j < 4 else d_v[...].reshape(1, D).astype(F32)
            col_v[j] = jnp.broadcast_to(row, (C, D)).T
        xs = [x_v[0, :, t * C:(t + 1) * C] for t in range(NT_)]
        sq, pv = {}, {}
        for u in ORDER0:
            if u == "W":
                wait(cp_w3)
                start(cp_step(5) + cp_step(6) + cp_step(7) + cp_last)
                _store_wide(wt_v, WV0, WV0 + D, wv_v[...].T)
                xs = [x_v[0, :, t * C:(t + 1) * C] for t in range(NT_)]
                continue
            op, r = u[:-1], int(u[-1])
            if op == "K":
                for t in range(NT_):
                    pk, sq[r, t] = k_unit(xs, r, t)
                    for e in range(2):
                        phik_v[2 * r + e, t] = pk[e].astype(BF16)
            elif op == "Q":
                for t in range(NT_):
                    q_unit(xs, 0, r, t, sq[r, t])
            elif op == "V":
                pv[r] = [v_unit(xs, 0, r, t) for t in range(NT_)]
            elif op == "KV":
                for g in (2 * r, 2 * r + 1):
                    kv_unit(g, [phik_v[g, t] for t in range(NT_)], pv[r], first=True)
            elif op == "FH":
                a_fwd_h(r, ab_l[r])
            elif op == "FU":
                a_fwd_u(r, ab_l[r])

    @pl.when((step >= 1) & (step < NB))
    def _():
        i = step
        wait(cp_step(step))
        glink[0] = None
        xs = [x_v[i, :, t * C:(t + 1) * C] for t in range(NT_)]
        n0 = 4 * (step - 1)
        pk, pv, sq, toks = {}, {}, {}, {}
        for u in ORDER1:
            op, r = u[:2], int(u[2])
            if op in ("K0", "K1"):
                t = int(op[1])
                pk[r, t], sq[r, t] = k_unit(xs, r, t)
                toks[u] = sq[r, t]
                toks["s" + u] = pk[r, t][1][136:144]
            elif op in ("V0", "V1"):
                pv[r, int(op[1])] = v_unit(xs, i, r, int(op[1]))
                toks[u] = pv[r, int(op[1])][0:8]
            elif op in ("Q0", "Q1"):
                toks[u] = q_unit(xs, i, r, int(op[1]), sq[r, int(op[1])])
            elif op in ("KA", "KB", "LA", "LB"):
                e = 0 if op[1] == "A" else 1
                kv_unit(2 * r + e, [pk[r, t][e] for t in range(NT_)], [pv[r, t] for t in range(NT_)],
                        part=1 if op[0] == "K" else 2)
            elif op == "FH":
                toks[u] = a_fwd_h(n0 + r + SKEW, ab_l[(r + SKEW) % 4])
            elif op == "FU":
                toks[u] = a_fwd_u(n0 + r + SKEW, ab_l[(r + SKEW) % 4])
            elif op == "IN":
                toks[u] = a_conv_inv(n0 + r, ab_l[r], {k: toks[v] for k, v in PACE[r].items()}, PSEQ[r])
        zls = [kvl_v[g, :, GR:GR + 1] for g in range(NG)]
        zmin = jnp.minimum(jnp.min(_tree(jnp.minimum, [kv_v[g, GR:GR + 1, :] for g in range(NG)]), keepdims=True),
                           jnp.min(_tree(jnp.minimum, zls), keepdims=True))
        zmax = jnp.max(_tree(jnp.maximum, zls), keepdims=True)
        ok_v[...] = jnp.broadcast_to(jnp.where(zmax <= 3.0 * zmin, 1.0, 0.0), (16, C))

    N2 = 4 * (NB - 1)

    @pl.when(step == NB)
    def _():
        wait(cp_last)
        glink[0] = None

        def head_of(v):
            return (v >= 18).astype(jnp.int32) + (v >= 36).astype(jnp.int32) + (v >= 54).astype(jnp.int32)

        r = _iota((80, C), 0)
        hr = jnp.where(r < GR, head_of(r), r & 3)
        mmask = hr == (_iota((80, C), 1) & 3)
        ll, lr = _iota((16, 80), 1), _iota((16, 80), 0)
        lmask = (head_of(ll) == (lr & 3)) & (ll < GR)
        hi4 = (lr & 4) != 0
        is17 = [lmask & hi4, lmask & jnp.logical_not(hi4)]
        sel = (((_iota((16, C), 1) >> 3) & 1) == (_iota((16, C), 0) >> 3)).astype(BF16)
        slow = ok_v[0, 0] < 0.5
        fast = ok_v[:, 0:80] > 0.5
        a_fwd_h(N2 + SKEW, ab_l[SKEW % 4])
        kvm = []
        for g in range(NG):
            kvl = kvl_v[g]
            k17 = jnp.where(is17[g % 2] & fast, kvl, 0.0).astype(BF16)
            tt = _dot(k17, sel, TN)
            kvm.append(jnp.where(mmask, kv_v[g] - tt, 0.0).astype(BF16))
            cb_v[g] = tt[0:GR] + pltpu.roll(tt[0:GR], 8, 1)
            k17f = jnp.where(is17[g % 2] & fast, kvl, 0.0).astype(BF16).astype(F32)
            k17f = jnp.concatenate([pltpu.roll(k17f[0:8], 4, 0), pltpu.roll(k17f[8:16], 4, 0)], axis=0)
            dd = jnp.where(is17[1 - g % 2], kvl - k17f, 0.0)
            dp_v[g // 2, :, GR * (g % 2):GR * (g % 2) + GR] = dd[:, 0:GR]
            zl_v[g] = jnp.broadcast_to(kvl[:, GR:GR + 1], (16, C))
        m16 = [_dot(dp_v[r_].astype(BF16), wo_v[144 * r_:144 * (r_ + 1), :]) for r_ in range(4)]
        a_fwd_u(N2 + SKEW, ab_l[SKEW % 4])
        wlast = jnp.concatenate([wo_v[4 * C:D, :].astype(F32)] + m16, axis=0)
        wot_v[KT - 1] = _pk(wlast.T)
        w4 = pltpu.bitcast(wo_v[0:4 * C, :].T, U32)
        for t in range(KT - 1):
            wot_v[t] = w4[:, t * C:(t + 1) * C]

        def num_unit(ct):
            omg = 1.0 - g_v[ct]
            for gp in range(NG // 2):
                os_, xs_ = [], []
                for e in range(2):
                    g = 2 * gp + e
                    nd = _dot(kvm[g], phiq_v[ct, g, 0:C, :])
                    pl_ = phiq_v[ct, g, C:2 * GR, :].astype(F32)
                    ph = [pl_[0:8], pl_[8:16]]
                    dl = ph[0] * zl_v[g, 0:8, :] + ph[1] * zl_v[g, 8:16, :]
                    den = nd[GR:GR + 8] + (dl + pltpu.roll(dl, 4, 0)) + 1e-6
                    rd = omg * pl.reciprocal(den, approx=True)
                    rd_v[ct, g] = rd
                    b = [jnp.broadcast_to(rd[j:j + 1], (8, C)) for j in range(4)]
                    pat = [b[0], b[0], jnp.where(lt2, b[0], b[1]), b[1], jnp.where(lt4, b[1], b[2]), b[2],
                           jnp.where(lt6, b[2], b[3]), b[3], b[3]]
                    os_ += [(nd[8 * j:8 * j + 8] + cb_v[g, 8 * j:8 * j + 8, :]) * pat[j] for j in range(9)]
                    xs_.append((ph, rd))
                ot_v[ct, 2 * GR * gp:2 * GR * (gp + 1), :] = jnp.concatenate(os_, axis=0).astype(BF16)
                rd = jnp.where(lt4, xs_[0][1], xs_[1][1])
                xx = [jnp.where(lt4, xs_[0][0][sg_], xs_[1][0][sg_]) * rd for sg_ in range(2)]
                ot_v[ct, D + 16 * gp:D + 16 * (gp + 1), :] = jnp.concatenate(xx, axis=0).astype(BF16)

        nstep = NCH + OLAG
        for it in range(nstep + 2 * NCH):
            if it < NCH:
                num_unit(it)
            if OLAG <= it < nstep:
                out_unit(0, it - OLAG)
            elif it >= nstep:
                out_unit(1 + (it - nstep) // NCH, (it - nstep) % NCH)
            if it >= nstep - 1 and (it - nstep + 1) % NCH == 0:
                out_copy((it - nstep + 1) // NCH).start()
            for n_ in range(8):
                if it == CPOS[n_]:
                    a_conv_inv(N2 + n_, ab_l[n_ % 4])
                if n_ < 4 and it == CPOS[n_] + FOFF[n_]:
                    a_fwd_h(N2 + n_ + 4, ab_l[n_ % 4])
                    a_fwd_u(N2 + n_ + 4, ab_l[n_ % 4])
        last = [out_copy(3, a, b, 3 + n_) for n_, (a, b) in enumerate(zip(LSPLIT[:-1], LSPLIT[1:]))]
        for ct in range(NCH):
            out_unit(3, ct)
            if ct + 1 in LSPLIT:
                last[LSPLIT.index(ct + 1) - 1].start()
        wait([out_copy(j) for j in range(3)] + last)

        @pl.when(slow)
        def _():
            for g in range(NG):
                dp_v[g // 2, :, GR * (g % 2):GR * (g % 2) + GR] = jnp.where(is17[g % 2], kvl_v[g], 0.0)[:, 0:GR]
            m17 = jnp.concatenate(
                [_dot(dp_v[r_].astype(BF16), wo_v[144 * r_:144 * (r_ + 1), :]) for r_ in range(4)],
                axis=0).astype(BF16)

            def body(ct, carry):
                xs_ = []
                for gp in range(NG // 2):
                    pa = phiq_v[ct, 2 * gp, C:2 * GR, :].astype(F32)
                    pb = phiq_v[ct, 2 * gp + 1, C:2 * GR, :].astype(F32)
                    rd = jnp.where(lt4, rd_v[ct, 2 * gp + 1], rd_v[ct, 2 * gp])
                    xs_ += [jnp.where(lt4, pb[8 * sg_:8 * sg_ + 8], pa[8 * sg_:8 * sg_ + 8]) * rd
                            for sg_ in range(2)]
                corr = _dot(m17, jnp.concatenate(xs_, axis=0).astype(BF16), TN)
                cols = pl.ds(pl.multiple_of(ct * C, C), C)
                o_v[:, cols] = (o_v[:, cols].astype(F32) + corr).astype(BF16)
                return carry

            lax.fori_loop(0, NCH, body, 0)
            again = pltpu.make_async_copy(o_v, o_hbm, sems.at[0])
            again.start()
            again.wait()


@jax.jit
def pallas_gated_mix__ssm_conv_h3__linear_kernel_hedgehog__prompt_kernel(A_q, A_k, A_v, A_shift_k, A_ssm_k, A_ssm_D, B_x, B_wqkv, B_w_phi, B_wo, gate_w):
    del B_x
    xt = jnp.transpose(A_q[0])
    kt = jnp.transpose(A_k[0])
    vt = jnp.transpose(A_v[0])
    sht = jnp.transpose(A_shift_k)
    wpt = jnp.transpose(B_w_phi, (1, 2, 0))
    out_t = pl.pallas_call(
        _kernel,
        grid=(NB + 1,),
        in_specs=[pl.BlockSpec(memory_space=pl.ANY)] * 10,
        out_specs=pl.BlockSpec(memory_space=pl.ANY),
        out_shape=jax.ShapeDtypeStruct((D, S), BF16),
        scratch_shapes=[
            pltpu.VMEM((NB, D, TS), BF16),
            pltpu.VMEM((D, S), BF16),
            pltpu.VMEM((D, S), BF16),
            pltpu.VMEM((D, S), BF16),
            pltpu.VMEM((4, D), BF16),
            pltpu.VMEM((D,), BF16),
            pltpu.VMEM((D, 9 * C), BF16),
            pltpu.VMEM((D, D), BF16),
            pltpu.VMEM((DH, DH, H), BF16),
            pltpu.VMEM((D, D), BF16),
            pltpu.VMEM((D,), BF16),
            pltpu.VMEM((2, 2, C // 2, C), U32),
            pltpu.VMEM((5, D, C), F32),
            pltpu.VMEM((DH, D), F32),
            pltpu.VMEM((KT, WROWS // 2, C), U32),
            pltpu.VMEM((KT, D // 2, C), U32),
            *[pltpu.VMEM((6, NCH, 16, C), F32) for _ in range(4)],
            pltpu.VMEM((NCH, D, C), F32),
            pltpu.VMEM((NCH, NG, 2 * GR, C), BF16),
            pltpu.VMEM((NG, NT_, 2 * GR, C), BF16),
            pltpu.VMEM((NCH, 8, C), F32),
            pltpu.VMEM((NG, 80, C), F32),
            pltpu.VMEM((NG, 16, 80), F32),
            pltpu.VMEM((NCH, KT * C, C), BF16),
            pltpu.VMEM((4, 16, 2 * GR), F32),
            pltpu.VMEM((NG, 16, C), F32),
            pltpu.VMEM((NG, GR, C), F32),
            pltpu.VMEM((D, S), BF16),
            pltpu.VMEM((NCH, NG, 8, C), F32),
            pltpu.VMEM((16, C), F32),
            pltpu.SemaphoreType.DMA((NB,)),
        ],
        compiler_params=pltpu.CompilerParams(
            dimension_semantics=("arbitrary",), vmem_limit_bytes=100 * 1024 * 1024),
    )(xt, kt, vt, sht, A_ssm_k, A_ssm_D, B_wqkv, wpt, B_wo, gate_w)
    return jnp.transpose(out_t)[None]
```
